```python
import jax
import jax.numpy as jnp

def _softmax(x, axis=-1):
    return jax.nn.softmax(x, axis=axis)

def _gelu(x):
    return jax.nn.gelu(x, approximate=True)

def _silu(x):
    return jax.nn.silu(x)

def _sigmoid(x):
    return jax.nn.sigmoid(x)

def _layernorm(x, axis=-1, eps=1e-05):
    m = jnp.mean(x, axis=axis, keepdims=True)
    v = jnp.var(x, axis=axis, keepdims=True)
    return (x - m) / jnp.sqrt(v + eps)

def _scatter_add(tgt, idx, src, axis=0):
    return tgt.at[idx].add(src)

def _segment_sum(src, seg, n):
    return jax.ops.segment_sum(src, seg, n)

class _Rng:

    def __init__(self, key):
        self._k = key

    def _next(self):
        self._k, sub = jax.random.split(self._k)
        return sub

    def normal(self, shape):
        return jax.random.normal(self._next(), shape, dtype=jnp.bfloat16)

    def randint(self, lo, hi, shape):
        return jax.random.randint(self._next(), shape, lo, hi, dtype=jnp.int32)

    def uniform(self, shape, lo=0.0, hi=1.0):
        return jax.random.uniform(self._next(), shape, jnp.bfloat16, lo, hi)

    def permutation(self, n):
        return jax.random.permutation(self._next(), n)
kernel_name = 'adaLN_cond__sliding_local_dilated__glu_gated_swiglu__prompt'

def setup_inputs():
    _rng = _Rng(jax.random.key(int.from_bytes(__import__("os").urandom(4), "little")))
    _w = lambda a: (lambda t: t.astype(jnp.bfloat16) if jnp.issubdtype(t.dtype, jnp.floating) else t)(jnp.asarray(a))

    def _A_setup():
        B, S, D = (1, 2048, 1024)
        return {'x': _w((lambda *s: _rng.normal(s) * 0.05)(B, S, D)), 'wqkv': _w((lambda *s: _rng.normal(s) * 0.05)(D, 3 * D)), 'wo': _w((lambda *s: _rng.normal(s) * 0.05)(D, D))}
    _A_in = _A_setup()

    def _B_setup():
        B, S, D, F = (1, 2048, 1024, 3584)
        return {'x': _w((lambda *s: _rng.normal(s) * 0.05)(B, S, D)), 'w1': _w((lambda *s: _rng.normal(s) * 0.05)(D, F) * (2.0 / D) ** 0.5), 'w3': _w((lambda *s: _rng.normal(s) * 0.05)(D, F) * (2.0 / D) ** 0.5), 'w2': _w((lambda *s: _rng.normal(s) * 0.05)(F, D) * (2.0 / F) ** 0.5)}
    _B_in = _B_setup()
    return {'A_x': _A_in['x'], 'A_wqkv': _A_in['wqkv'], 'A_wo': _A_in['wo'], 'B_x': _B_in['x'], 'B_w1': _B_in['w1'], 'B_w3': _B_in['w3'], 'B_w2': _B_in['w2'], 'c': _w((lambda *s: _rng.normal(s) * 0.05)(1, 1024)), 'w_mod': _w((lambda *s: _rng.normal(s) * 0.05)(1024, 6 * 1024) * 1024 ** (-0.5))}

def reference(A_x, A_wqkv, A_wo, B_x, B_w1, B_w3, B_w2, c, w_mod):

    def _A_ref(x, wqkv, wo):
        B, S, D = x.shape
        H = 32
        Dh = D // H
        W, dil = (8, 2)
        qkv = (lambda x, *d: x.transpose(*d))((x @ wqkv).reshape(B, S, 3, H, Dh), 2, 0, 3, 1, 4)
        q, k, v = (qkv[0], qkv[1], qkv[2])
        scale = Dh ** (-0.5)
        pos = jnp.arange(S)
        off = jnp.arange(W) * dil
        idx = pos[:, None] - off[None, :]
        mask = idx >= 0
        idx_c = jnp.where(mask, idx, 0).reshape(-1)
        kg = k[:, :, idx_c, :].reshape(B, H, S, W, Dh)
        vg = v[:, :, idx_c, :].reshape(B, H, S, W, Dh)
        logits = jnp.einsum('bhsd,bhswd->bhsw', q, kg) * scale
        logits = jnp.where(mask[None, None, :, :], logits, -1000000000.0)
        attn = _softmax(logits, axis=-1)
        o = jnp.einsum('bhsw,bhswd->bhsd', attn, vg)
        return (lambda x, *d: x.transpose(*d))(o, 0, 2, 1, 3).reshape(B, S, D) @ wo

    def _B_ref(x, w1, w3, w2):
        gate = jnp.einsum('bsd,df->bsf', x, w1)
        up = jnp.einsum('bsd,df->bsf', x, w3)
        h = _silu(gate) * up
        out = jnp.einsum('bsf,fd->bsd', h, w2)
        return out
    x = A_x
    mod = (_silu(c) @ w_mod).reshape(c.shape[0], 6, 1, -1)
    sa, ca, ga, sb, cb, gb = (mod[:, 0].copy(), mod[:, 1].copy(), mod[:, 2].copy(), mod[:, 3].copy(), mod[:, 4].copy(), mod[:, 5].copy())
    h = _layernorm(x, axis=-1) * (1 + ca) + sa
    x = x + ga * _A_ref(h, A_wqkv, A_wo)
    h = _layernorm(x, axis=-1) * (1 + cb) + sb
    x = x + gb * _B_ref(h, B_w1, B_w3, B_w2)
    return x
```

```python
import functools, math
import jax, jax.numpy as jnp
from jax import lax
from jax.experimental import pallas as pl
from jax.experimental.pallas import tpu as pltpu

S, D, F, H, Dh, W, DIL = 2048, 1024, 3584, 32, 32, 8, 2
PAD = 16
bf16, f32 = jnp.bfloat16, jnp.float32
QSCALE = Dh ** -0.5 * math.log2(math.e)

def _ln_mod(x, scale1, shift):
    m = jnp.mean(x, axis=-1, keepdims=True)
    xc = x - m
    v = jnp.mean(xc * xc, axis=-1, keepdims=True)
    return xc * lax.rsqrt(v + 1e-5) * scale1 + shift

def make(TM=256, R=16, TF=512, TM2=256, UNROLL1=True):
    NB = S // TM

    def kern(x_hbm, wqkv_hbm, wo_hbm, w1_hbm, w3_hbm, w2_hbm, c_hbm, wmod_hbm, out_hbm,
             x_v, wqkv_v, wp_v, wo_v, wop_v, w1_v, w3_v, w2_v, c_v, wmod_v, kS, vS, qS, oS, x1_v, h2_v, h1_v, out_v, mod_v,
             sems, osems):
        cp = lambda src, dst, i: pltpu.make_async_copy(src, dst, sems.at[i])
        d_c = cp(c_hbm, c_v, 0)
        d_wma = cp(wmod_hbm.at[:, 0:2 * D], wmod_v.at[:, 0:2 * D], 1)
        d_x = cp(x_hbm, x_v, 2)
        d_wqkv = cp(wqkv_hbm, wqkv_v, 3)
        d_wo = cp(wo_hbm, wo_v, 4)
        d_wmb = cp(wmod_hbm.at[:, 2 * D:6 * D], wmod_v.at[:, 2 * D:6 * D], 5)
        d_w1 = cp(w1_hbm, w1_v, 6)
        d_w3 = cp(w3_hbm, w3_v, 7)
        d_w2 = cp(w2_hbm, w2_v, 8)
        d_c.start(); d_wma.start(); d_x.start(); d_wqkv.start()
        kS[:, 0:PAD, :] = jnp.zeros((8, PAD, 128), f32)
        vS[:, 0:PAD, :] = jnp.zeros((8, PAD, 128), f32)
        d_c.wait(); d_wma.wait()
        d_wo.start(); d_wmb.start()
        cf = c_v[...].astype(f32)
        sc = jnp.broadcast_to((cf * jax.nn.sigmoid(cf)).astype(bf16), (16, D))
        mod_v[:, 0:2 * D] = jnp.dot(sc, wmod_v[:, 0:2 * D], preferred_element_type=f32)[0:8]
        d_wqkv.wait()
        d_w1.start(); d_w3.start(); d_w2.start()
        for t in range(3):
            for g in range(8):
                col = t * D + g * 128
                wt = wqkv_v[:, col:col + 128].T
                for c in range(8):
                    piece = jnp.concatenate([wt[32 * a + 4 * c:32 * a + 4 * c + 4, :] for a in range(4)], axis=0)
                    r0 = t * D + c * 128 + g * 16
                    wp_v[r0:r0 + 16, :] = piece
        d_x.wait()

        def ln1(i):
            rows = pl.ds(i * TM, TM)
            sa = mod_v[:, 0:D][0:1]; ca = mod_v[:, D:2 * D][0:1]
            h1_v[rows, :] = _ln_mod(x_v[rows, :].astype(f32), 1.0 + ca, sa).astype(bf16)

        def qkv(i):
            r0 = i * TM
            r = lax.dot_general(h1_v[pl.ds(r0, TM), :], wp_v[...], (((1,), (1,)), ((), ())), preferred_element_type=f32)
            for c in range(8):
                qS[c, pl.ds(r0, TM), :] = r[:, c * 128:(c + 1) * 128] * QSCALE
                kS[c, pl.ds(PAD + r0, TM), :] = r[:, D + c * 128:D + (c + 1) * 128]
                vS[c, pl.ds(PAD + r0, TM), :] = r[:, 2 * D + c * 128:2 * D + (c + 1) * 128]

        lane = lax.broadcasted_iota(jnp.int32, (R, 128), 1)
        ix1, ix2 = lane ^ 1, lane ^ 2

        def att(i):
            for r in range(TM // R):
                r0 = i * TM + r * R
                q = [qS[c, pl.ds(r0, R), :] for c in range(8)]
                lg = []
                for w in range(W):
                    p = q[0] * kS[0, pl.ds(PAD + r0 - DIL * w, R), :]
                    for c in range(1, 8):
                        p = p + q[c] * kS[c, pl.ds(PAD + r0 - DIL * w, R), :]
                    p = p + jnp.take_along_axis(p, ix1, axis=1)
                    p = p + jnp.take_along_axis(p, ix2, axis=1)
                    if isinstance(r0, int) and r0 < DIL * w:
                        row = lax.broadcasted_iota(jnp.int32, (R, 128), 0) + r0
                        p = jnp.where(row >= DIL * w, p, -1e9 * math.log2(math.e))
                    lg.append(p)
                m = functools.reduce(jnp.maximum, lg)
                e = [jnp.exp2(l - m) for l in lg]
                inv = 1.0 / functools.reduce(lambda a, b: a + b, e)
                for c in range(8):
                    o = e[0] * vS[c, pl.ds(PAD + r0, R), :]
                    for w in range(1, W):
                        o = o + e[w] * vS[c, pl.ds(PAD + r0 - DIL * w, R), :]
                    oS[pl.ds(r0, R), c * 128:(c + 1) * 128] = (o * inv).astype(bf16)

        def wo_ln2(i):
            rows = pl.ds(i * TM, TM)
            ga = mod_v[:, 2 * D:3 * D][0:1]; sb = mod_v[:, 3 * D:4 * D][0:1]; cb = mod_v[:, 4 * D:5 * D][0:1]
            a = jnp.dot(oS[rows, :], wop_v[...], preferred_element_type=f32)
            x1 = x_v[rows, :].astype(f32) + ga * a
            x1_v[rows, :] = x1
            h2_v[rows, :] = _ln_mod(x1, 1.0 + cb, sb).astype(bf16)

        def prep_late():
            d_wo.wait(); d_wmb.wait()
            mod_v[:, 2 * D:6 * D] = jnp.dot(sc, wmod_v[:, 2 * D:6 * D], preferred_element_type=f32)[0:8]
            for g in range(8):
                wt = wo_v[g * 128:(g + 1) * 128, :]
                for c in range(8):
                    piece = jnp.concatenate([wt[32 * a + 4 * c:32 * a + 4 * c + 4, :] for a in range(4)], axis=0)
                    wop_v[c * 128 + g * 16:c * 128 + g * 16 + 16, :] = piece

        ln1(0); ln1(1)
        qkv(0)
        prep_late()
        for i in range(NB - 1):
            qkv(i + 1)
            if i + 2 < NB: ln1(i + 2)
            att(i)
            wo_ln2(i)
        att(NB - 1)
        wo_ln2(NB - 1)

        d_w1.wait(); d_w3.wait(); d_w2.wait()
        NB2 = S // TM2

        def ffn(i, carry):
            rows = pl.ds(pl.multiple_of(i * TM2, TM2), TM2)
            h = h2_v[rows, :]
            acc = jnp.zeros((TM2, D), f32)
            for f in range(F // TF):
                fs = slice(f * TF, (f + 1) * TF)
                g = jnp.dot(h, w1_v[:, fs], preferred_element_type=f32)
                u = jnp.dot(h, w3_v[:, fs], preferred_element_type=f32)
                a = (g * jax.nn.sigmoid(g) * u).astype(bf16)
                acc = acc + jnp.dot(a, w2_v[fs, :], preferred_element_type=f32)
            gb = mod_v[:, 5 * D:6 * D][0:1]
            out_v[rows, :] = (x1_v[rows, :] + gb * acc).astype(bf16)
            pltpu.make_async_copy(out_v.at[rows, :], out_hbm.at[rows, :], osems.at[i]).start()
            return carry
        lax.fori_loop(0, NB2, ffn, 0)
        for i in range(NB2):
            rows = pl.ds(i * TM2, TM2)
            pltpu.make_async_copy(out_v.at[rows, :], out_hbm.at[rows, :], osems.at[i]).wait()

    V = pltpu.VMEM
    scratch = [V((S, D), bf16), V((D, 3 * D), bf16), V((3 * D, D), bf16), V((D, D), bf16), V((D, D), bf16),
               V((D, F), bf16), V((D, F), bf16), V((F, D), bf16), V((1, D), bf16), V((D, 6 * D), bf16),
               V((8, PAD + S, 128), f32), V((8, PAD + S, 128), f32), V((8, S, 128), f32), V((S, D), bf16),
               V((S, D), f32), V((S, D), bf16), V((S, D), bf16), V((S, D), bf16), V((8, 6 * D), f32),
               pltpu.SemaphoreType.DMA((9,)), pltpu.SemaphoreType.DMA((S // TM2,))]
    call = pl.pallas_call(kern, out_shape=jax.ShapeDtypeStruct((S, D), bf16),
                          in_specs=[pl.BlockSpec(memory_space=pl.ANY)] * 8, out_specs=pl.BlockSpec(memory_space=pl.ANY),
                          scratch_shapes=scratch,
                          compiler_params=pltpu.CompilerParams(vmem_limit_bytes=120 * 1024 * 1024))

    def fn(A_x, A_wqkv, A_wo, B_x, B_w1, B_w3, B_w2, c, w_mod):
        return call(A_x.reshape(S, D), A_wqkv, A_wo, B_w1, B_w3, B_w2, c, w_mod).reshape(1, S, D)
    return fn


_KERNEL = make()


@jax.jit
def pallas_adaLN_cond__sliding_local_dilated__glu_gated_swiglu__prompt_kernel(
    A_x, A_wqkv, A_wo, B_x, B_w1, B_w3, B_w2, c, w_mod
):
    return _KERNEL(A_x, A_wqkv, A_wo, B_x, B_w1, B_w3, B_w2, c, w_mod)
```

```python
import functools, math, contextlib
import jax, jax.numpy as jnp
from jax import lax
from jax.experimental import pallas as pl
from jax.experimental.pallas import tpu as pltpu

S, D, F, H, Dh, W, DIL = 2048, 1024, 3584, 32, 32, 8, 2
PAD = 16
bf16, f32, i32 = jnp.bfloat16, jnp.float32, jnp.int32
QSCALE = Dh ** -0.5 * math.log2(math.e)
NEG = -1e9 * math.log2(math.e)
NT = (((1,), (1,)), ((), ()))


def make(TM=256, R=8, TF=512, CHAIN=1, LNCH=2, SCOPES=False, NA=4, PREPCH=0, MODCH=4, TOKM=0, TREE=0, TIE=0, LN2LOOP=1):
    NB = S // TM
    scope = (lambda n: jax.named_scope(n)) if SCOPES else (lambda n: contextlib.nullcontext())

    def kern(x_hbm, wqkv_hbm, wo_hbm, w1_hbm, w3_hbm, w2_hbm, c_hbm, wmod_hbm, out_hbm,
             x_v, wqkv_v, wp_v, wo_v, wop_v, w1_v, w3_v, w2_v, c_v, wmod_v, kS, vS, qS, oS, x1_v, h_v, out_v, mod_v,
             sems, osems):
        cnt = [0]
        def cp(src, dst):
            cnt[0] += 1
            return pltpu.make_async_copy(src, dst, sems.at[cnt[0] - 1])
        XA = 3 * TM
        d_c = cp(c_hbm, c_v)
        d_xa = cp(x_hbm.at[0:XA, :], x_v.at[0:XA, :])
        d_wv = cp(wqkv_hbm.at[:, 2 * D:3 * D], wqkv_v.at[:, 2 * D:3 * D])
        MW = 2 * D // MODCH
        d_wma = [cp(wmod_hbm.at[:, j * MW:(j + 1) * MW], wmod_v.at[:, j * MW:(j + 1) * MW]) for j in range(MODCH)]
        d_xb = cp(x_hbm.at[XA:S, :], x_v.at[XA:S, :])
        d_wk = cp(wqkv_hbm.at[:, D:2 * D], wqkv_v.at[:, D:2 * D])
        d_wq = cp(wqkv_hbm.at[:, 0:D], wqkv_v.at[:, 0:D])
        d_wo = cp(wo_hbm, wo_v)
        d_wmb = cp(wmod_hbm.at[:, 2 * D:6 * D], wmod_v.at[:, 2 * D:6 * D])
        d_w1 = cp(w1_hbm, w1_v)
        d_w3 = cp(w3_hbm, w3_v)
        d_w2 = cp(w2_hbm, w2_v)
        for d in [d_c, d_xa, d_wv] + d_wma + [d_xb, d_wk, d_wq, d_wo, d_wmb, d_w1, d_w3, d_w2]:
            d.start()
        kS[:, 0:PAD, :] = jnp.zeros((8, PAD, 128), f32)
        vS[:, 0:PAD, :] = jnp.zeros((8, PAD, 128), f32)

        def prep_w(t):
            for g in range(8):
                col = t * D + g * 128
                wt = wqkv_v[:, col:col + 128].T
                for c in range(8):
                    piece = jnp.concatenate([wt[32 * a + 4 * c:32 * a + 4 * c + 4, :] for a in range(4)], axis=0)
                    r0 = t * D + c * 128 + g * 16
                    wp_v[r0:r0 + 16, :] = piece

        def prep_wo():
            for g in range(8):
                wt = wo_v[g * 128:(g + 1) * 128, :]
                for c in range(8):
                    piece = jnp.concatenate([wt[32 * a + 4 * c:32 * a + 4 * c + 4, :] for a in range(4)], axis=0)
                    wop_v[c * 128 + g * 16:c * 128 + g * 16 + 16, :] = piece

        def two(v):
            return jnp.concatenate([v, v], axis=0)

        def ln_core(x, scale1, shift):
            m = jnp.sum(x, axis=-1, keepdims=True) * (1.0 / D)
            xc = x - m
            v = jnp.sum(xc * xc, axis=-1, keepdims=True) * (1.0 / D)
            rs = lax.rsqrt(v + 1e-5)
            return (xc * rs * two(scale1) + two(shift)).astype(bf16), rs

        ln_tok = []
        def gate_of(tok):
            return jnp.where(jnp.broadcast_to(tok[0:8], (8, 128)) > -1.0, 0, 1).astype(i32)

        def ln1(i, gated=True):
            for r in range(TM // 16):
                r0 = i * TM + r * 16
                xb = x_v[r0:r0 + 16, :]
                if gated and LNCH and len(ln_tok) >= LNCH:
                    g = gate_of(ln_tok[-LNCH])
                    xb = pltpu.bitcast(pltpu.bitcast(xb, i32) | jnp.concatenate([g] * 8, axis=1), bf16)
                h, rs = ln_core(xb.astype(f32), mod_v[:, D:2 * D], mod_v[:, 0:D])
                ln_tok.append(rs)
                h_v[r0:r0 + 16, :] = h

        def ln2_chunk(i, r, tok=None):
            r0 = i * TM + r * 16
            if not isinstance(r0, int): r0 = pl.multiple_of(r0, 16)
            x = x1_v[pl.ds(r0, 16), :]
            if tok is not None:
                gz = jnp.where(jnp.broadcast_to(tok[0:8], (8, 128)) > -1.0, 0.0, 1.0)
                x = x + two(jnp.concatenate([gz] * 8, axis=1))
            h, rs = ln_core(x, mod_v[:, 4 * D:5 * D], mod_v[:, 3 * D:4 * D])
            h_v[pl.ds(r0, 16), :] = h
            return rs

        def ln2(i):
            tok = []
            for r in range(TM // 16):
                tok.append(ln2_chunk(i, r, tok[-LNCH] if (LNCH and len(tok) >= LNCH) else None))

        def proj(i, t, dst, pad):
            r0 = i * TM
            r = lax.dot_general(h_v[r0:r0 + TM, :], wp_v[t * D:(t + 1) * D, :], NT, preferred_element_type=f32)
            for c in range(8):
                dst[c, pad + r0:pad + r0 + TM, :] = r[:, c * 128:(c + 1) * 128]

        lane = lax.broadcasted_iota(i32, (R, 128), 1)
        ix1, ix2 = lane ^ 1, lane ^ 2
        chain = []
        def att(i, tie=None):
            for r in range(TM // R):
                r0 = i * TM + r * R
                cond = None
                if CHAIN and len(chain) >= CHAIN:
                    cond = chain[-CHAIN] > -1.0
                if tie is not None and (r * R) % 16 == 0:
                    t2 = jnp.broadcast_to(ln2_chunk(tie, (r * R) // 16)[0:8], (8, 128)) > -1.0
                    if R == 16: t2 = jnp.concatenate([t2, t2], axis=0)
                    cond = t2 if cond is None else jnp.logical_and(cond, t2)
                qs = QSCALE if cond is None else jnp.where(cond, QSCALE, QSCALE * (1 + 2.0 ** -20))
                q = [qS[c, r0:r0 + R, :] * qs for c in range(8)]
                lg = []
                for w in range(W):
                    b0 = PAD + r0 - DIL * w
                    p = q[0] * kS[0, b0:b0 + R, :]
                    for c in range(1, 8):
                        p = p + q[c] * kS[c, b0:b0 + R, :]
                    p = p + jnp.take_along_axis(p, ix1, axis=1)
                    p = p + jnp.take_along_axis(p, ix2, axis=1)
                    if r0 < DIL * w:
                        row = lax.broadcasted_iota(i32, (R, 128), 0) + r0
                        p = jnp.where(row >= DIL * w, p, NEG)
                    lg.append(p)
                if TREE:
                    m = jnp.maximum(jnp.maximum(jnp.maximum(lg[0], lg[1]), jnp.maximum(lg[2], lg[3])), jnp.maximum(jnp.maximum(lg[4], lg[5]), jnp.maximum(lg[6], lg[7])))
                else:
                    m = functools.reduce(jnp.maximum, lg)
                e = [jnp.exp2(l - m) for l in lg]
                if TREE:
                    den = ((e[0] + e[1]) + (e[2] + e[3])) + ((e[4] + e[5]) + (e[6] + e[7]))
                else:
                    den = functools.reduce(lambda a, b: a + b, e)
                inv = 1.0 / den
                chain.append(e[0] if TOKM == 1 else (den if TOKM == 2 else inv))
                for c in range(8):
                    o = e[0] * vS[c, PAD + r0:PAD + r0 + R, :]
                    for w in range(1, W):
                        b0 = PAD + r0 - DIL * w
                        o = o + e[w] * vS[c, b0:b0 + R, :]
                    oS[r0:r0 + R, c * 128:(c + 1) * 128] = (o * inv).astype(bf16)

        def wo_mm(i):
            r0 = i * TM
            a = jnp.dot(oS[r0:r0 + TM, :], wop_v[...], preferred_element_type=f32)
            ga = mod_v[:, 2 * D:3 * D]
            x1_v[r0:r0 + TM, :] = x_v[r0:r0 + TM, :].astype(f32) + jnp.concatenate([ga] * (TM // 8), axis=0) * a

        def ffn_part(rows, chunks, mid=None):
            h = h_v[rows, :]
            acc = None
            for n, f in enumerate(chunks):
                if mid is not None and n == mid[0]:
                    mid[1]()
                fs = slice(f * TF, (f + 1) * TF)
                g = jnp.dot(h, w1_v[:, fs], preferred_element_type=f32)
                u = jnp.dot(h, w3_v[:, fs], preferred_element_type=f32)
                a = (g * jax.nn.sigmoid(g) * u).astype(bf16)
                y = jnp.dot(a, w2_v[fs, :], preferred_element_type=f32)
                acc = y if acc is None else acc + y
            return acc

        with scope('w_xa_wv'):
            d_xa.wait(); d_wv.wait()
        with scope('prep_v'):
            prep_w(2)
        with scope('w_c'):
            d_c.wait()
        cf = c_v[...].astype(f32)
        sc = jnp.broadcast_to((cf * jax.nn.sigmoid(cf)).astype(bf16), (16, D))
        with scope('mod_a'):
            for j in range(MODCH):
                d_wma[j].wait()
                r = jnp.dot(sc, wmod_v[:, j * MW:(j + 1) * MW], preferred_element_type=f32)[0:8]
                if j * MW >= D:
                    r = r + 1.0
                mod_v[:, j * MW:(j + 1) * MW] = r
        with scope('R2'):
            ln1(0, gated=False)
            proj(0, 2, vS, PAD)
            ln1(1); ln1(2)
            proj(1, 2, vS, PAD)
        with scope('w_xb_wk'):
            d_xb.wait(); d_wk.wait()
        with scope('R3'):
            for i in range(3, NB): ln1(i)
            for i in range(2, NB): proj(i, 2, vS, PAD)
            prep_w(1)
        with scope('w_wq_wo_wmb'):
            d_wq.wait(); d_wo.wait(); d_wmb.wait()
        with scope('R4'):
            prep_w(0)
            proj(0, 1, kS, PAD)
            r = jnp.dot(sc, wmod_v[:, 2 * D:6 * D], preferred_element_type=f32)[0:8]
            mod_v[:, 2 * D:4 * D] = r[:, 0:2 * D]
            mod_v[:, 4 * D:5 * D] = r[:, 2 * D:3 * D] + 1.0
            mod_v[:, 5 * D:6 * D] = r[:, 3 * D:4 * D]
            prep_wo()
            proj(0, 0, qS, 0)
            for i in range(1, NB - 1):
                proj(i, 1, kS, PAD)
                proj(i, 0, qS, 0)
                att(i - 1, tie=(i - 2) if (TIE and i >= 2) else None)
                wo_mm(i - 1)
                if LN2LOOP:
                    if i == 1: ln2(0)
                elif not TIE: ln2(i - 1)
            i = NB - 1
            att(i - 1, tie=(i - 2) if TIE else None)
            proj(i, 1, kS, PAD)
            wo_mm(i - 1)
            if not TIE and not LN2LOOP: ln2(i - 1)
            proj(i, 0, qS, 0)
        with scope('w_ffn'):
            d_w1.wait(); d_w3.wait(); d_w2.wait()
        NC = F // TF
        gb = mod_v[:, 5 * D:6 * D]
        gbt = jnp.concatenate([gb] * (TM // 8), axis=0)
        with scope('R5'):
            att(NB - 1, tie=(NB - 2) if TIE else None)
            def mid():
                wo_mm(NB - 1)
                if not LN2LOOP: ln2(NB - 1)
            if LN2LOOP: ln2(1)
            acc = ffn_part(slice(0, TM), range(0, NA), mid=(NA // 2, mid))
            x1_v[0:TM, :] = x1_v[0:TM, :] + gbt * acc

        def loopA(i, carry):
            rows = pl.ds(pl.multiple_of(i * TM, TM), TM)
            acc = ffn_part(rows, range(0, NA))
            if LN2LOOP: ln2(jnp.minimum(i + 1, NB - 1))
            gbt = jnp.concatenate([mod_v[:, 5 * D:6 * D]] * (TM // 8), axis=0)
            x1_v[rows, :] = x1_v[rows, :] + gbt * acc
            return carry
        with scope('loopA'):
            lax.fori_loop(1, NB, loopA, 0)

        def loopB(i, carry):
            rows = pl.ds(pl.multiple_of(i * TM, TM), TM)
            acc = ffn_part(rows, range(NA, NC))
            gbt = jnp.concatenate([mod_v[:, 5 * D:6 * D]] * (TM // 8), axis=0)
            out_v[rows, :] = (x1_v[rows, :] + gbt * acc).astype(bf16)
            pltpu.make_async_copy(out_v.at[rows, :], out_hbm.at[rows, :], osems.at[i]).start()
            return carry
        with scope('loopB'):
            lax.fori_loop(0, NB, loopB, 0)
        with scope('tail'):
            for i in range(NB):
                rows = pl.ds(i * TM, TM)
                pltpu.make_async_copy(out_v.at[rows, :], out_hbm.at[rows, :], osems.at[i]).wait()

    V = pltpu.VMEM
    scratch = [V((S, D), bf16), V((D, 3 * D), bf16), V((3 * D, D), bf16), V((D, D), bf16), V((D, D), bf16),
               V((D, F), bf16), V((D, F), bf16), V((F, D), bf16), V((1, D), bf16), V((D, 6 * D), bf16),
               V((8, PAD + S, 128), f32), V((8, PAD + S, 128), f32), V((8, S, 128), f32), V((S, D), bf16),
               V((S, D), f32), V((S, D), bf16), V((S, D), bf16), V((8, 6 * D), f32),
               pltpu.SemaphoreType.DMA((11 + MODCH,)), pltpu.SemaphoreType.DMA((NB,))]
    call = pl.pallas_call(kern, out_shape=jax.ShapeDtypeStruct((S, D), bf16),
                          in_specs=[pl.BlockSpec(memory_space=pl.ANY)] * 8, out_specs=pl.BlockSpec(memory_space=pl.ANY),
                          scratch_shapes=scratch,
                          compiler_params=pltpu.CompilerParams(vmem_limit_bytes=120 * 1024 * 1024))

    def fn(A_x, A_wqkv, A_wo, B_x, B_w1, B_w3, B_w2, c, w_mod):
        return call(A_x.reshape(S, D), A_wqkv, A_wo, B_w1, B_w3, B_w2, c, w_mod).reshape(1, S, D)
    return fn


_KERNEL = make(CHAIN=2, TOKM=1, TREE=1)


@jax.jit
def pallas_adaLN_cond__sliding_local_dilated__glu_gated_swiglu__prompt_kernel(
    A_x, A_wqkv, A_wo, B_x, B_w1, B_w3, B_w2, c, w_mod
):
    return _KERNEL(A_x, A_wqkv, A_wo, B_x, B_w1, B_w3, B_w2, c, w_mod)
```

```python
import functools, math, contextlib
import jax, jax.numpy as jnp
from jax import lax
from jax.experimental import pallas as pl
from jax.experimental.pallas import tpu as pltpu

S, D, F, H, Dh, W, DIL = 2048, 1024, 3584, 32, 32, 8, 2
PAD = 16
bf16, f32, i32 = jnp.bfloat16, jnp.float32, jnp.int32
QSCALE = Dh ** -0.5 * math.log2(math.e)
NEG = -1e9 * math.log2(math.e)
NT = (((1,), (1,)), ((), ()))
NANBITS = 0x7FC17FC1


def make(TM=256, R=8, TF=512, CHAIN=2, LNCH=2, LNCH1=2, SCOPES=False, NA=4, MODI=2, NS=3,
         TIE_WO=0, TIE_LN=0, TIE_PK=0, HK=512):
    NB = S // TM
    scope = (lambda n: jax.named_scope(n)) if SCOPES else (lambda n: contextlib.nullcontext())

    def kern(x_hbm, wqkv_hbm, wo_hbm, w1_hbm, w3_hbm, w2_hbm, c_hbm, wmod_hbm, out_hbm,
             x_v, wqkv_v, wp_v, wo_v, wop_v, w1_v, w3_v, w2_v, c_v, wmod_v, kS, vS, qS, oS, x1_v, h_v, out_v, mod_v,
             sems, osems):
        cnt = [0]
        def cp(src, dst):
            cnt[0] += 1
            return pltpu.make_async_copy(src, dst, sems.at[cnt[0] - 1])
        def cp2(src, dst, idx):
            return cp(src.at[idx], dst.at[idx])
        A_, B_ = slice(0, HK), slice(HK, D)
        d_c = cp(c_hbm, c_v)
        d_xa = cp2(x_hbm, x_v, (slice(0, NS * TM), slice(None)))
        d_wva = cp2(wqkv_hbm, wqkv_v, (A_, slice(2 * D, 3 * D)))
        d_ma = [cp2(wmod_hbm, wmod_v, (slice(None), slice(o + A_.start, o + A_.stop))) for o in (D, 0)]
        d_wvb = cp2(wqkv_hbm, wqkv_v, (B_, slice(2 * D, 3 * D)))
        d_mb = [cp2(wmod_hbm, wmod_v, (slice(None), slice(o + B_.start, o + B_.stop))) for o in (D, 0)]
        d_xn = cp2(x_hbm, x_v, (slice(NS * TM, (NS + 1) * TM), slice(None)))
        d_xb = cp2(x_hbm, x_v, (slice((NS + 1) * TM, S), slice(None)))
        d_wk = cp2(wqkv_hbm, wqkv_v, (slice(None), slice(D, 2 * D)))
        d_wq = cp2(wqkv_hbm, wqkv_v, (slice(None), slice(0, D)))
        d_wo = cp(wo_hbm, wo_v)
        d_wmb = cp2(wmod_hbm, wmod_v, (slice(None), slice(2 * D, 6 * D)))
        d_w1 = cp(w1_hbm, w1_v)
        d_w3 = cp(w3_hbm, w3_v)
        d_w2 = cp(w2_hbm, w2_v)
        for d in [d_c, d_xa, d_wva] + d_ma + [d_wvb] + d_mb + [d_xn, d_xb, d_wk, d_wq, d_wo, d_wmb, d_w1, d_w3, d_w2]:
            d.start()
        kS[:, 0:PAD, :] = jnp.zeros((8, PAD, 128), f32)
        vS[:, 0:PAD, :] = jnp.zeros((8, PAD, 128), f32)

        def nan_gate(vals):
            ok = None
            for v in vals:
                t = pltpu.bitcast(v[0:16, 0:128], i32) != NANBITS
                ok = t if ok is None else jnp.logical_and(ok, t)
            return jnp.where(ok, 0, 1).astype(i32)

        def or_gate(vb, g):
            n, m = vb.shape[0] // 16, vb.shape[1] // 128
            gg = jnp.concatenate([g] * m, axis=1) if m > 1 else g
            gg = jnp.concatenate([gg] * n, axis=0) if n > 1 else gg
            return pltpu.bitcast(pltpu.bitcast(vb, i32) | gg, bf16)

        def prep_w(t, ks=slice(0, D), gate=None):
            out = []
            for g in range(8):
                col = t * D + g * 128
                wt = wqkv_v[ks, col:col + 128].T
                for c in range(8):
                    piece = jnp.concatenate([wt[32 * a + 4 * c:32 * a + 4 * c + 4, :] for a in range(4)], axis=0)
                    if gate is not None and g == 7 and c == 7:
                        piece = or_gate(piece, gate)
                    r0 = t * D + c * 128 + g * 16
                    wp_v[r0:r0 + 16, ks] = piece
                    out.append(piece)
            return out

        def prep_wo():
            out = []
            for g in range(8):
                wt = wo_v[g * 128:(g + 1) * 128, :]
                for c in range(8):
                    piece = jnp.concatenate([wt[32 * a + 4 * c:32 * a + 4 * c + 4, :] for a in range(4)], axis=0)
                    wop_v[c * 128 + g * 16:c * 128 + g * 16 + 16, :] = piece
                    out.append(piece)
            return out

        def two(v):
            return jnp.concatenate([v, v], axis=0)

        def ln_norm(x):
            m = jnp.sum(x, axis=-1, keepdims=True) * (1.0 / D)
            xc = x - m
            v = jnp.sum(xc * xc, axis=-1, keepdims=True) * (1.0 / D)
            rs = lax.rsqrt(v + 1e-5)
            return xc * rs, rs

        def tok_ok(tok):
            return jnp.broadcast_to(tok[0:8], (8, 128)) > -1.0

        ln_tok = []
        def ln1(i):
            for r in range(TM // 16):
                r0 = i * TM + r * 16
                xb = x_v[r0:r0 + 16, :]
                if LNCH1 and len(ln_tok) >= LNCH1:
                    xb = or_gate(xb, jnp.where(tok_ok(ln_tok[-LNCH1]), 0, 1).astype(i32))
                n, rs = ln_norm(xb.astype(f32))
                ln_tok.append(rs)
                h_v[r0:r0 + 16, :] = (n * two(mod_v[:, D:2 * D]) + two(mod_v[:, 0:D])).astype(bf16)

        def ln1_stats(i):
            for r in range(TM // 16):
                r0 = i * TM + r * 16
                n, _ = ln_norm(x_v[r0:r0 + 16, :].astype(f32))
                for c in range(8):
                    qS[c, r0:r0 + 16, :] = n[:, c * 128:(c + 1) * 128]

        def ln1_half(i, ks):
            r0 = i * TM
            for c in range(ks.start // 128, ks.stop // 128):
                cs = slice(c * 128, (c + 1) * 128)
                s1 = jnp.concatenate([mod_v[:, D + c * 128:D + (c + 1) * 128]] * (TM // 8), axis=0)
                sh = jnp.concatenate([mod_v[:, c * 128:(c + 1) * 128]] * (TM // 8), axis=0)
                h_v[r0:r0 + TM, cs] = (qS[c, r0:r0 + TM, :] * s1 + sh).astype(bf16)

        def ln2(i):
            tok = []
            for r in range(TM // 16):
                r0 = i * TM + r * 16
                if not isinstance(r0, int): r0 = pl.multiple_of(r0, 16)
                x = x1_v[pl.ds(r0, 16), :]
                if LNCH and len(tok) >= LNCH:
                    gz = jnp.where(tok_ok(tok[-LNCH]), 0.0, 1.0)
                    x = x + two(jnp.concatenate([gz] * 8, axis=1))
                n, rs = ln_norm(x)
                h_v[pl.ds(r0, 16), :] = (n * two(mod_v[:, 4 * D:5 * D]) + two(mod_v[:, 3 * D:4 * D])).astype(bf16)
                tok.append(rs)
            return tok

        def proj(i, t, dst, pad, ks=None, add=False, gate=None):
            r0 = i * TM
            ks = ks or slice(0, D)
            h = h_v[r0:r0 + TM, ks]
            if gate is not None: h = or_gate(h, gate)
            r = lax.dot_general(h, wp_v[t * D:(t + 1) * D, ks], NT, preferred_element_type=f32)
            for c in range(8):
                rr = r[:, c * 128:(c + 1) * 128]
                if add: rr = rr + dst[c, pad + r0:pad + r0 + TM, :]
                dst[c, pad + r0:pad + r0 + TM, :] = rr

        def proj_mod(i, t, dst, pad, sc, tiles):
            r0 = i * TM
            h = h_v[r0:r0 + TM, :]
            for c in range(8):
                wt = wp_v[t * D + c * 128:t * D + (c + 1) * 128, :]
                j = tiles[c]
                hk = D // 2
                r = lax.dot_general(h[:, :hk], wt[:, :hk], NT, preferred_element_type=f32)
                m = jnp.dot(sc[:, :hk], wmod_v[0:hk, j * 128:(j + 1) * 128], preferred_element_type=f32)
                r = r + lax.dot_general(h[:, hk:], wt[:, hk:], NT, preferred_element_type=f32)
                m = m + jnp.dot(sc[:, hk:], wmod_v[hk:, j * 128:(j + 1) * 128], preferred_element_type=f32)
                dst[c, pad + r0:pad + r0 + TM, :] = r
                m = m[0:8]
                if 4 * 8 <= j < 5 * 8: m = m + 1.0
                mod_v[:, j * 128:(j + 1) * 128] = m

        lane = lax.broadcasted_iota(i32, (R, 128), 1)
        ix1, ix2 = lane ^ 1, lane ^ 2
        chain = []
        def att(i):
            for r in range(TM // R):
                r0 = i * TM + r * R
                qs = QSCALE
                if CHAIN and len(chain) >= CHAIN:
                    qs = jnp.where(chain[-CHAIN] > -1.0, QSCALE, QSCALE * (1 + 2.0 ** -20))
                q = [qS[c, r0:r0 + R, :] * qs for c in range(8)]
                lg = []
                for w in range(W):
                    b0 = PAD + r0 - DIL * w
                    p = q[0] * kS[0, b0:b0 + R, :]
                    for c in range(1, 8):
                        p = p + q[c] * kS[c, b0:b0 + R, :]
                    p = p + jnp.take_along_axis(p, ix1, axis=1)
                    p = p + jnp.take_along_axis(p, ix2, axis=1)
                    if r0 < DIL * w:
                        row = lax.broadcasted_iota(i32, (R, 128), 0) + r0
                        p = jnp.where(row >= DIL * w, p, NEG)
                    lg.append(p)
                mx = jnp.maximum
                m = mx(mx(mx(lg[0], lg[1]), mx(lg[2], lg[3])), mx(mx(lg[4], lg[5]), mx(lg[6], lg[7])))
                e = [jnp.exp2(l - m) for l in lg]
                den = ((e[0] + e[1]) + (e[2] + e[3])) + ((e[4] + e[5]) + (e[6] + e[7]))
                inv = 1.0 / den
                chain.append(e[0])
                for c in range(8):
                    o = e[0] * vS[c, PAD + r0:PAD + r0 + R, :]
                    for w in range(1, W):
                        b0 = PAD + r0 - DIL * w
                        o = o + e[w] * vS[c, b0:b0 + R, :]
                    oS[r0:r0 + R, c * 128:(c + 1) * 128] = (o * inv).astype(bf16)

        def wo_mm(i):
            r0 = i * TM
            a = jnp.dot(oS[r0:r0 + TM, :], wop_v[...], preferred_element_type=f32)
            ga = mod_v[:, 2 * D:3 * D]
            x1_v[r0:r0 + TM, :] = x_v[r0:r0 + TM, :].astype(f32) + jnp.concatenate([ga] * (TM // 8), axis=0) * a

        def ffn_part(rows, chunks, mid=None):
            h = h_v[rows, :]
            acc = None
            for n, f in enumerate(chunks):
                if mid is not None and n == mid[0]:
                    mid[1]()
                fs = slice(f * TF, (f + 1) * TF)
                g = jnp.dot(h, w1_v[:, fs], preferred_element_type=f32)
                u = jnp.dot(h, w3_v[:, fs], preferred_element_type=f32)
                a = (g * jax.nn.sigmoid(g) * u).astype(bf16)
                y = jnp.dot(a, w2_v[fs, :], preferred_element_type=f32)
                acc = y if acc is None else acc + y
            return acc

        def mod_half(sc, dmas, ks):
            for o, d in zip((D, 0), dmas):
                d.wait()
                r = jnp.dot(sc, wmod_v[:, o + ks.start:o + ks.stop], preferred_element_type=f32)[0:8]
                mod_v[:, o + ks.start:o + ks.stop] = r + 1.0 if o == D else r

        with scope('w_xa'):
            d_xa.wait()
        with scope('stats'):
            for i in range(NS): ln1_stats(i)
        with scope('w_wva'):
            d_wva.wait()
        with scope('prep_va'):
            prep_w(2, A_)
        with scope('mod_a'):
            d_c.wait()
            cf = c_v[...].astype(f32)
            sc = jnp.broadcast_to((cf * jax.nn.sigmoid(cf)).astype(bf16), (16, D))
            mod_half(sc, d_ma, A_)
        with scope('RA'):
            ln1_half(0, A_)
            proj(0, 2, vS, PAD, A_)
            d_wvb.wait()
            prep_w(2, B_)
            for i in range(1, NS):
                ln1_half(i, A_)
                proj(i, 2, vS, PAD, A_)
        with scope('mod_b'):
            mod_half(sc, d_mb, B_)
            d_xn.wait()
        with scope('RB'):
            for i in range(NS):
                ln1_half(i, B_)
                proj(i, 2, vS, PAD, B_, add=True)
            ln1(NS)
        with scope('w_xb_wk'):
            d_xb.wait(); d_wk.wait()
        with scope('R3'):
            for i in range(NS + 1, NB): ln1(i)
            prep_w(1)
            for i in range(NS, NB): proj(i, 2, vS, PAD)
            proj(0, 1, kS, PAD)
            proj(1, 1, kS, PAD)
        with scope('w_wq_wo_wmb'):
            d_wq.wait(); d_wo.wait(); d_wmb.wait()
        with scope('R4'):
            pw = prep_wo()
            prep_w(0, gate=nan_gate(pw) if TIE_WO else None)
            proj_mod(2, 1, kS, PAD, sc, range(16, 24))
            proj_mod(0, 0, qS, 0, sc, range(24, 32))
            ltok = None
            for i in range(1, NB):
                if i == 1:
                    proj_mod(3, 1, kS, PAD, sc, range(32, 40))
                    proj_mod(1, 0, qS, 0, sc, range(40, 48))
                else:
                    if i + 2 < NB:
                        gate = None
                        if TIE_LN and i + 2 == TIE_LN:
                            ok = functools.reduce(jnp.logical_and, [tok_ok(t) for t in ltok[-max(LNCH, 1):]])
                            gate = jnp.where(ok, 0, 1).astype(i32)
                        proj(i + 2, 1, kS, PAD, gate=gate)
                    proj(i, 0, qS, 0)
                att(i - 1)
                wo_mm(i - 1)
                if i == 1: ltok = ln2(0)
        with scope('w_ffn'):
            d_w1.wait(); d_w3.wait(); d_w2.wait()
        NC = F // TF
        with scope('R5'):
            att(NB - 1)
            ln2(1)
            acc = ffn_part(slice(0, TM), range(0, NA), mid=(NA // 2, lambda: wo_mm(NB - 1)))
            gbt = jnp.concatenate([mod_v[:, 5 * D:6 * D]] * (TM // 8), axis=0)
            x1_v[0:TM, :] = x1_v[0:TM, :] + gbt * acc

        def loopA(i, carry):
            rows = pl.ds(pl.multiple_of(i * TM, TM), TM)
            acc = ffn_part(rows, range(0, NA))
            ln2(jnp.minimum(i + 1, NB - 1))
            gbt = jnp.concatenate([mod_v[:, 5 * D:6 * D]] * (TM // 8), axis=0)
            x1_v[rows, :] = x1_v[rows, :] + gbt * acc
            return carry
        with scope('loopA'):
            lax.fori_loop(1, NB, loopA, 0)

        def loopB(i, carry):
            rows = pl.ds(pl.multiple_of(i * TM, TM), TM)
            acc = ffn_part(rows, range(NA, NC))
            gbt = jnp.concatenate([mod_v[:, 5 * D:6 * D]] * (TM // 8), axis=0)
            out_v[rows, :] = (x1_v[rows, :] + gbt * acc).astype(bf16)
            pltpu.make_async_copy(out_v.at[rows, :], out_hbm.at[rows, :], osems.at[i]).start()
            return carry
        with scope('loopB'):
            lax.fori_loop(0, NB, loopB, 0)
        with scope('tail'):
            for i in range(NB):
                rows = pl.ds(i * TM, TM)
                pltpu.make_async_copy(out_v.at[rows, :], out_hbm.at[rows, :], osems.at[i]).wait()

    V = pltpu.VMEM
    scratch = [V((S, D), bf16), V((D, 3 * D), bf16), V((3 * D, D), bf16), V((D, D), bf16), V((D, D), bf16),
               V((D, F), bf16), V((D, F), bf16), V((F, D), bf16), V((1, D), bf16), V((D, 6 * D), bf16),
               V((8, PAD + S, 128), f32), V((8, PAD + S, 128), f32), V((8, S, 128), f32), V((S, D), bf16),
               V((S, D), f32), V((S, D), bf16), V((S, D), bf16), V((8, 6 * D), f32),
               pltpu.SemaphoreType.DMA((17,)), pltpu.SemaphoreType.DMA((NB,))]
    call = pl.pallas_call(kern, out_shape=jax.ShapeDtypeStruct((S, D), bf16),
                          in_specs=[pl.BlockSpec(memory_space=pl.ANY)] * 8, out_specs=pl.BlockSpec(memory_space=pl.ANY),
                          scratch_shapes=scratch,
                          compiler_params=pltpu.CompilerParams(vmem_limit_bytes=120 * 1024 * 1024))

    def fn(A_x, A_wqkv, A_wo, B_x, B_w1, B_w3, B_w2, c, w_mod):
        return call(A_x.reshape(S, D), A_wqkv, A_wo, B_w1, B_w3, B_w2, c, w_mod).reshape(1, S, D)
    return fn


_KERNEL = make()


@jax.jit
def pallas_adaLN_cond__sliding_local_dilated__glu_gated_swiglu__prompt_kernel(
    A_x, A_wqkv, A_wo, B_x, B_w1, B_w3, B_w2, c, w_mod
):
    return _KERNEL(A_x, A_wqkv, A_wo, B_x, B_w1, B_w3, B_w2, c, w_mod)
```

```python
import functools, math, contextlib
import jax, jax.numpy as jnp
from jax import lax
from jax.experimental import pallas as pl
from jax.experimental.pallas import tpu as pltpu

S, D, F, H, Dh, W, DIL = 2048, 1024, 3584, 32, 32, 8, 2
PAD = 16
bf16, f32, i32 = jnp.bfloat16, jnp.float32, jnp.int32
QSCALE = Dh ** -0.5 * math.log2(math.e)
NEG = -1e9 * math.log2(math.e)
NT = (((1,), (1,)), ((), ()))
NANBITS = 0x7FC17FC1


def make(TM=256, R=8, TF=512, CHAIN=2, LNCH=2, LNCH1=2, SCOPES=False, NA=4, MODI=2, NS=3,
         TIE_WO=0, TIE_LN=0, TIE_PK=0, KSP=4, NV1=1, KL=2, CHL=None, NCL=2, NOFFNDMA=0):
    NB = S // TM
    scope = (lambda n: jax.named_scope(n)) if SCOPES else (lambda n: contextlib.nullcontext())

    def kern(x_hbm, wqkv_hbm, wo_hbm, w1_hbm, w3_hbm, w2_hbm, c_hbm, wmod_hbm, out_hbm,
             x_v, wqkv_v, wp_v, wo_v, wop_v, w1_v, w3_v, w2_v, c_v, wmod_v, kS, vS, qS, oS, x1_v, h_v, out_v, mod_v,
             sems, osems):
        cnt = [0]
        def cp(src, dst):
            cnt[0] += 1
            return pltpu.make_async_copy(src, dst, sems.at[cnt[0] - 1])
        def cp2(src, dst, idx):
            return cp(src.at[idx], dst.at[idx])
        KQ = [slice(j * D // KSP, (j + 1) * D // KSP) for j in range(KSP)]
        d_c = cp(c_hbm, c_v)
        d_xa = cp2(x_hbm, x_v, (slice(0, NS * TM), slice(None)))
        d_wv = [cp2(wqkv_hbm, wqkv_v, (ks, slice(2 * D, 3 * D))) for ks in KQ]
        d_m = [[cp2(wmod_hbm, wmod_v, (slice(None), slice(o + ks.start, o + ks.stop))) for o in (D, 0)] for ks in KQ]
        d_xn = cp2(x_hbm, x_v, (slice(NS * TM, (NS + 1) * TM), slice(None)))
        d_xb = cp2(x_hbm, x_v, (slice((NS + 1) * TM, S), slice(None)))
        d_wk = cp2(wqkv_hbm, wqkv_v, (slice(None), slice(D, 2 * D)))
        d_wq = cp2(wqkv_hbm, wqkv_v, (slice(None), slice(0, D)))
        d_wo = cp(wo_hbm, wo_v)
        d_wmb = cp2(wmod_hbm, wmod_v, (slice(None), slice(2 * D, 6 * D)))
        d_w1 = cp(w1_hbm, w1_v)
        d_w3 = cp(w3_hbm, w3_v)
        d_w2 = cp(w2_hbm, w2_v)
        first = [d_c, d_xa]
        for j in range(KSP): first += [d_wv[j]] + d_m[j]
        for d in first + [d_xn, d_xb, d_wk, d_wq, d_wo, d_wmb] + ([] if NOFFNDMA else [d_w1, d_w3, d_w2]):
            d.start()
        kS[:, 0:PAD, :] = jnp.zeros((8, PAD, 128), f32)
        vS[:, 0:PAD, :] = jnp.zeros((8, PAD, 128), f32)

        def nan_gate(vals):
            ok = None
            for v in vals:
                t = pltpu.bitcast(v[0:16, 0:128], i32) != NANBITS
                ok = t if ok is None else jnp.logical_and(ok, t)
            return jnp.where(ok, 0, 1).astype(i32)

        def or_gate(vb, g):
            n, m = vb.shape[0] // 16, vb.shape[1] // 128
            gg = jnp.concatenate([g] * m, axis=1) if m > 1 else g
            gg = jnp.concatenate([gg] * n, axis=0) if n > 1 else gg
            return pltpu.bitcast(pltpu.bitcast(vb, i32) | gg, bf16)

        def prep_w(t, ks=slice(0, D), gate=None):
            out = []
            for g in range(8):
                col = t * D + g * 128
                wt = wqkv_v[ks, col:col + 128].T
                for c in range(8):
                    piece = jnp.concatenate([wt[32 * a + 4 * c:32 * a + 4 * c + 4, :] for a in range(4)], axis=0)
                    if gate is not None and g == 7 and c == 7:
                        piece = or_gate(piece, gate)
                    r0 = t * D + c * 128 + g * 16
                    wp_v[r0:r0 + 16, ks] = piece
                    out.append(piece)
            return out

        def prep_wo():
            out = []
            for g in range(8):
                wt = wo_v[g * 128:(g + 1) * 128, :]
                for c in range(8):
                    piece = jnp.concatenate([wt[32 * a + 4 * c:32 * a + 4 * c + 4, :] for a in range(4)], axis=0)
                    wop_v[c * 128 + g * 16:c * 128 + g * 16 + 16, :] = piece
                    out.append(piece)
            return out

        def two(v):
            return jnp.concatenate([v, v], axis=0)

        def ln_norm(x):
            m = jnp.sum(x, axis=-1, keepdims=True) * (1.0 / D)
            xc = x - m
            v = jnp.sum(xc * xc, axis=-1, keepdims=True) * (1.0 / D)
            rs = lax.rsqrt(v + 1e-5)
            return xc * rs, rs

        def tok_ok(tok):
            return jnp.broadcast_to(tok[0:8], (8, 128)) > -1.0

        ln_tok = []
        def ln1(i):
            for r in range(TM // 16):
                r0 = i * TM + r * 16
                xb = x_v[r0:r0 + 16, :]
                if LNCH1 and len(ln_tok) >= LNCH1:
                    xb = or_gate(xb, jnp.where(tok_ok(ln_tok[-LNCH1]), 0, 1).astype(i32))
                n, rs = ln_norm(xb.astype(f32))
                ln_tok.append(rs)
                h_v[r0:r0 + 16, :] = (n * two(mod_v[:, D:2 * D]) + two(mod_v[:, 0:D])).astype(bf16)

        def ln1_stats(i):
            for r in range(TM // 16):
                r0 = i * TM + r * 16
                n, _ = ln_norm(x_v[r0:r0 + 16, :].astype(f32))
                for c in range(8):
                    qS[c, r0:r0 + 16, :] = n[:, c * 128:(c + 1) * 128]

        def ln1_half(i, ks):
            r0 = i * TM
            for c in range(ks.start // 128, ks.stop // 128):
                cs = slice(c * 128, (c + 1) * 128)
                s1 = jnp.concatenate([mod_v[:, D + c * 128:D + (c + 1) * 128]] * (TM // 8), axis=0)
                sh = jnp.concatenate([mod_v[:, c * 128:(c + 1) * 128]] * (TM // 8), axis=0)
                h_v[r0:r0 + TM, cs] = (qS[c, r0:r0 + TM, :] * s1 + sh).astype(bf16)

        def ln2(i):
            tok = []
            for r in range(TM // 16):
                r0 = i * TM + r * 16
                if not isinstance(r0, int): r0 = pl.multiple_of(r0, 16)
                x = x1_v[pl.ds(r0, 16), :]
                if LNCH and len(tok) >= LNCH:
                    gz = jnp.where(tok_ok(tok[-LNCH]), 0.0, 1.0)
                    x = x + two(jnp.concatenate([gz] * 8, axis=1))
                n, rs = ln_norm(x)
                h_v[pl.ds(r0, 16), :] = (n * two(mod_v[:, 4 * D:5 * D]) + two(mod_v[:, 3 * D:4 * D])).astype(bf16)
                tok.append(rs)
            return tok

        def proj(i, t, dst, pad, ks=None, add=False, gate=None):
            r0 = i * TM
            ks = ks or slice(0, D)
            h = h_v[r0:r0 + TM, ks]
            if gate is not None: h = or_gate(h, gate)
            r = lax.dot_general(h, wp_v[t * D:(t + 1) * D, ks], NT, preferred_element_type=f32)
            for c in range(8):
                rr = r[:, c * 128:(c + 1) * 128]
                if add: rr = rr + dst[c, pad + r0:pad + r0 + TM, :]
                dst[c, pad + r0:pad + r0 + TM, :] = rr

        def proj_mod(i, t, dst, pad, sc, tiles):
            r0 = i * TM
            h = h_v[r0:r0 + TM, :]
            for c in range(8):
                wt = wp_v[t * D + c * 128:t * D + (c + 1) * 128, :]
                j = tiles[c]
                hk = D // 2
                r = lax.dot_general(h[:, :hk], wt[:, :hk], NT, preferred_element_type=f32)
                m = jnp.dot(sc[:, :hk], wmod_v[0:hk, j * 128:(j + 1) * 128], preferred_element_type=f32)
                r = r + lax.dot_general(h[:, hk:], wt[:, hk:], NT, preferred_element_type=f32)
                m = m + jnp.dot(sc[:, hk:], wmod_v[hk:, j * 128:(j + 1) * 128], preferred_element_type=f32)
                dst[c, pad + r0:pad + r0 + TM, :] = r
                m = m[0:8]
                if 4 * 8 <= j < 5 * 8: m = m + 1.0
                mod_v[:, j * 128:(j + 1) * 128] = m

        lane = lax.broadcasted_iota(i32, (R, 128), 1)
        ix1, ix2 = lane ^ 1, lane ^ 2
        chain = []
        def att(i):
            ch = CHL if (CHL and NB - 1 - NCL <= i < NB - 1) else CHAIN
            for r in range(TM // R):
                r0 = i * TM + r * R
                qs = QSCALE
                if ch and len(chain) >= ch:
                    qs = jnp.where(chain[-ch] > -1.0, QSCALE, QSCALE * (1 + 2.0 ** -20))
                q = [qS[c, r0:r0 + R, :] * qs for c in range(8)]
                lg = []
                for w in range(W):
                    b0 = PAD + r0 - DIL * w
                    p = q[0] * kS[0, b0:b0 + R, :]
                    for c in range(1, 8):
                        p = p + q[c] * kS[c, b0:b0 + R, :]
                    p = p + jnp.take_along_axis(p, ix1, axis=1)
                    p = p + jnp.take_along_axis(p, ix2, axis=1)
                    if r0 < DIL * w:
                        row = lax.broadcasted_iota(i32, (R, 128), 0) + r0
                        p = jnp.where(row >= DIL * w, p, NEG)
                    lg.append(p)
                mx = jnp.maximum
                m = mx(mx(mx(lg[0], lg[1]), mx(lg[2], lg[3])), mx(mx(lg[4], lg[5]), mx(lg[6], lg[7])))
                e = [jnp.exp2(l - m) for l in lg]
                den = ((e[0] + e[1]) + (e[2] + e[3])) + ((e[4] + e[5]) + (e[6] + e[7]))
                inv = 1.0 / den
                chain.append(e[0])
                for c in range(8):
                    o = e[0] * vS[c, PAD + r0:PAD + r0 + R, :]
                    for w in range(1, W):
                        b0 = PAD + r0 - DIL * w
                        o = o + e[w] * vS[c, b0:b0 + R, :]
                    oS[r0:r0 + R, c * 128:(c + 1) * 128] = (o * inv).astype(bf16)

        def wo_mm(i):
            r0 = i * TM
            a = jnp.dot(oS[r0:r0 + TM, :], wop_v[...], preferred_element_type=f32)
            ga = mod_v[:, 2 * D:3 * D]
            x1_v[r0:r0 + TM, :] = x_v[r0:r0 + TM, :].astype(f32) + jnp.concatenate([ga] * (TM // 8), axis=0) * a

        def ffn_part(rows, chunks, mid=None):
            h = h_v[rows, :]
            acc = None
            for n, f in enumerate(chunks):
                if mid is not None and n == mid[0]:
                    mid[1]()
                fs = slice(f * TF, (f + 1) * TF)
                g = jnp.dot(h, w1_v[:, fs], preferred_element_type=f32)
                u = jnp.dot(h, w3_v[:, fs], preferred_element_type=f32)
                a = (g * jax.nn.sigmoid(g) * u).astype(bf16)
                y = jnp.dot(a, w2_v[fs, :], preferred_element_type=f32)
                acc = y if acc is None else acc + y
            return acc

        def mod_half(sc, dmas, ks):
            for d in dmas: d.wait()
            for o in (D, 0):
                r = jnp.dot(sc, wmod_v[:, o + ks.start:o + ks.stop], preferred_element_type=f32)[0:8]
                mod_v[:, o + ks.start:o + ks.stop] = r + 1.0 if o == D else r

        with scope('w_xa'):
            d_xa.wait()
        with scope('stats'):
            for i in range(NS): ln1_stats(i)
        with scope('w_wva'):
            d_wv[0].wait()
        with scope('prep_va'):
            prep_w(2, KQ[0])
        d_c.wait()
        cf = c_v[...].astype(f32)
        sc = jnp.broadcast_to((cf * jax.nn.sigmoid(cf)).astype(bf16), (16, D))
        for j in range(KSP):
            with scope(f'mod{j}'):
                mod_half(sc, d_m[j], KQ[j])
                if j == KSP - 1: d_xn.wait()
            with scope(f'RV{j}'):
                ln1_half(0, KQ[j])
                proj(0, 2, vS, PAD, KQ[j], add=j > 0)
                if j + 1 < KSP:
                    d_wv[j + 1].wait()
                    prep_w(2, KQ[j + 1])
                for i in range(1, NS):
                    ln1_half(i, KQ[j])
                    proj(i, 2, vS, PAD, KQ[j], add=j > 0)
                if j == KSP - 1: ln1(NS)
        with scope('w_xb'):
            d_xb.wait()
        with scope('R3'):
            for i in range(NS + 1, NS + NV1 + 1): ln1(i)
            for i in range(NS, NS + NV1): proj(i, 2, vS, PAD)
            d_wk.wait()
            for i in range(NS + NV1 + 1, NB): ln1(i)
            prep_w(1)
            for i in range(NS + NV1, NB): proj(i, 2, vS, PAD)
            for i in range(KL): proj(i, 1, kS, PAD)
        with scope('w_wq_wo_wmb'):
            d_wq.wait(); d_wo.wait(); d_wmb.wait()
        with scope('R4'):
            pw = prep_wo()
            prep_w(0, gate=nan_gate(pw) if TIE_WO else None)
            proj_mod(KL, 1, kS, PAD, sc, range(16, 24))
            proj_mod(0, 0, qS, 0, sc, range(24, 32))
            ltok = None
            for i in range(1, NB):
                if i == 1:
                    proj_mod(1 + KL, 1, kS, PAD, sc, range(32, 40))
                    proj_mod(1, 0, qS, 0, sc, range(40, 48))
                else:
                    if i + KL < NB:
                        gate = None
                        if TIE_LN and i + KL == TIE_LN:
                            ok = functools.reduce(jnp.logical_and, [tok_ok(t) for t in ltok[-max(LNCH, 1):]])
                            gate = jnp.where(ok, 0, 1).astype(i32)
                        proj(i + KL, 1, kS, PAD, gate=gate)
                    proj(i, 0, qS, 0)
                att(i - 1)
                wo_mm(i - 1)
                if i == 1: ltok = ln2(0)
        with scope('w_ffn'):
            if NOFFNDMA: d_w1.start(); d_w3.start(); d_w2.start()
            d_w1.wait(); d_w3.wait(); d_w2.wait()
        NC = F // TF
        with scope('R5'):
            att(NB - 1)
            ln2(1)
            acc = ffn_part(slice(0, TM), range(0, NA), mid=(NA // 2, lambda: wo_mm(NB - 1)))
            gbt = jnp.concatenate([mod_v[:, 5 * D:6 * D]] * (TM // 8), axis=0)
            x1_v[0:TM, :] = x1_v[0:TM, :] + gbt * acc

        def loopA(i, carry):
            rows = pl.ds(pl.multiple_of(i * TM, TM), TM)
            acc = ffn_part(rows, range(0, NA))
            ln2(jnp.minimum(i + 1, NB - 1))
            gbt = jnp.concatenate([mod_v[:, 5 * D:6 * D]] * (TM // 8), axis=0)
            x1_v[rows, :] = x1_v[rows, :] + gbt * acc
            return carry
        with scope('loopA'):
            lax.fori_loop(1, NB, loopA, 0)

        def loopB(i, carry):
            rows = pl.ds(pl.multiple_of(i * TM, TM), TM)
            acc = ffn_part(rows, range(NA, NC))
            gbt = jnp.concatenate([mod_v[:, 5 * D:6 * D]] * (TM // 8), axis=0)
            out_v[rows, :] = (x1_v[rows, :] + gbt * acc).astype(bf16)
            pltpu.make_async_copy(out_v.at[rows, :], out_hbm.at[rows, :], osems.at[i]).start()
            return carry
        with scope('loopB'):
            lax.fori_loop(0, NB, loopB, 0)
        with scope('tail'):
            for i in range(NB):
                rows = pl.ds(i * TM, TM)
                pltpu.make_async_copy(out_v.at[rows, :], out_hbm.at[rows, :], osems.at[i]).wait()

    V = pltpu.VMEM
    scratch = [V((S, D), bf16), V((D, 3 * D), bf16), V((3 * D, D), bf16), V((D, D), bf16), V((D, D), bf16),
               V((D, F), bf16), V((D, F), bf16), V((F, D), bf16), V((1, D), bf16), V((D, 6 * D), bf16),
               V((8, PAD + S, 128), f32), V((8, PAD + S, 128), f32), V((8, S, 128), f32), V((S, D), bf16),
               V((S, D), f32), V((S, D), bf16), V((S, D), bf16), V((8, 6 * D), f32),
               pltpu.SemaphoreType.DMA((11 + 3 * KSP,)), pltpu.SemaphoreType.DMA((NB,))]
    call = pl.pallas_call(kern, out_shape=jax.ShapeDtypeStruct((S, D), bf16),
                          in_specs=[pl.BlockSpec(memory_space=pl.ANY)] * 8, out_specs=pl.BlockSpec(memory_space=pl.ANY),
                          scratch_shapes=scratch,
                          compiler_params=pltpu.CompilerParams(vmem_limit_bytes=120 * 1024 * 1024))

    def fn(A_x, A_wqkv, A_wo, B_x, B_w1, B_w3, B_w2, c, w_mod):
        return call(A_x.reshape(S, D), A_wqkv, A_wo, B_w1, B_w3, B_w2, c, w_mod).reshape(1, S, D)
    return fn


_KERNEL = make()


@jax.jit
def pallas_adaLN_cond__sliding_local_dilated__glu_gated_swiglu__prompt_kernel(
    A_x, A_wqkv, A_wo, B_x, B_w1, B_w3, B_w2, c, w_mod
):
    return _KERNEL(A_x, A_wqkv, A_wo, B_x, B_w1, B_w3, B_w2, c, w_mod)
```

```python
import functools, math, contextlib
import jax, jax.numpy as jnp
from jax import lax
from jax.experimental import pallas as pl
from jax.experimental.pallas import tpu as pltpu

S, D, F, H, Dh, W, DIL = 2048, 1024, 3584, 32, 32, 8, 2
PAD = 16
bf16, f32, i32 = jnp.bfloat16, jnp.float32, jnp.int32
QSCALE = Dh ** -0.5 * math.log2(math.e)
NEG = -1e9 * math.log2(math.e)
NT = (((1,), (1,)), ((), ()))
NANBITS = 0x7FC17FC1


def make(TM=256, R=8, TF=512, CHAIN=2, LNCH=2, LNCH1=2, SCOPES=False, NA=4, MODI=2, NS=3,
         TIE_WO=0, TIE_LN=0, TIE_PK=0, KSP=4, NV1=3, EARLYPREP=1, MODV=0, MODCHN=1, KL=2, CHL=None, NCL=2, NOFFNDMA=0):
    NB = S // TM
    scope = (lambda n: jax.named_scope(n)) if SCOPES else (lambda n: contextlib.nullcontext())

    def kern(x_hbm, wqkv_hbm, wo_hbm, w1_hbm, w3_hbm, w2_hbm, c_hbm, wmod_hbm, out_hbm,
             x_v, wqkv_v, wp_v, wo_v, wop_v, w1_v, w3_v, w2_v, c_v, wmod_v, kS, vS, qS, oS, x1_v, h_v, out_v, mod_v, scT_v,
             sems, osems):
        cnt = [0]
        def cp(src, dst):
            cnt[0] += 1
            return pltpu.make_async_copy(src, dst, sems.at[cnt[0] - 1])
        def cp2(src, dst, idx):
            return cp(src.at[idx], dst.at[idx])
        KQ = [slice(j * D // KSP, (j + 1) * D // KSP) for j in range(KSP)]
        d_c = cp(c_hbm, c_v)
        d_xa = cp2(x_hbm, x_v, (slice(0, NS * TM), slice(None)))
        d_wv = [cp2(wqkv_hbm, wqkv_v, (ks, slice(2 * D, 3 * D))) for ks in KQ]
        d_m = [[cp2(wmod_hbm, wmod_v, (slice(None), slice(o + ks.start, o + ks.stop))) for o in (D, 0)] for ks in KQ]
        d_xn = cp2(x_hbm, x_v, (slice(NS * TM, (NS + 1) * TM), slice(None)))
        d_xb = cp2(x_hbm, x_v, (slice((NS + 1) * TM, S), slice(None)))
        d_wk = cp2(wqkv_hbm, wqkv_v, (slice(None), slice(D, 2 * D)))
        d_wq = cp2(wqkv_hbm, wqkv_v, (slice(None), slice(0, D)))
        d_wo = cp(wo_hbm, wo_v)
        d_wmb = cp2(wmod_hbm, wmod_v, (slice(None), slice(2 * D, 6 * D)))
        d_w1 = cp(w1_hbm, w1_v)
        d_w3 = cp(w3_hbm, w3_v)
        d_w2 = cp(w2_hbm, w2_v)
        first = [d_c, d_xa]
        for j in range(KSP): first += [d_wv[j]] + d_m[j]
        for d in first + [d_xn, d_xb, d_wk, d_wq, d_wo, d_wmb] + ([] if NOFFNDMA else [d_w1, d_w3, d_w2]):
            d.start()
        kS[:, 0:PAD, :] = jnp.zeros((8, PAD, 128), f32)
        vS[:, 0:PAD, :] = jnp.zeros((8, PAD, 128), f32)

        def nan_gate(vals):
            ok = None
            for v in vals:
                t = pltpu.bitcast(v[0:16, 0:128], i32) != NANBITS
                ok = t if ok is None else jnp.logical_and(ok, t)
            return jnp.where(ok, 0, 1).astype(i32)

        def or_gate(vb, g):
            n, m = vb.shape[0] // 16, vb.shape[1] // 128
            gg = jnp.concatenate([g] * m, axis=1) if m > 1 else g
            gg = jnp.concatenate([gg] * n, axis=0) if n > 1 else gg
            return pltpu.bitcast(pltpu.bitcast(vb, i32) | gg, bf16)

        def prep_w(t, ks=slice(0, D), gate=None):
            out = []
            for g in range(8):
                col = t * D + g * 128
                wt = wqkv_v[ks, col:col + 128].T
                for c in range(8):
                    piece = jnp.concatenate([wt[32 * a + 4 * c:32 * a + 4 * c + 4, :] for a in range(4)], axis=0)
                    if gate is not None and g == 7 and c == 7:
                        piece = or_gate(piece, gate)
                    r0 = t * D + c * 128 + g * 16
                    wp_v[r0:r0 + 16, ks] = piece
                    out.append(piece)
            return out

        def prep_wo():
            out = []
            for g in range(8):
                wt = wo_v[g * 128:(g + 1) * 128, :]
                for c in range(8):
                    piece = jnp.concatenate([wt[32 * a + 4 * c:32 * a + 4 * c + 4, :] for a in range(4)], axis=0)
                    wop_v[c * 128 + g * 16:c * 128 + g * 16 + 16, :] = piece
                    out.append(piece)
            return out

        def two(v):
            return jnp.concatenate([v, v], axis=0)

        def ln_norm(x):
            m = jnp.sum(x, axis=-1, keepdims=True) * (1.0 / D)
            xc = x - m
            v = jnp.sum(xc * xc, axis=-1, keepdims=True) * (1.0 / D)
            rs = lax.rsqrt(v + 1e-5)
            return xc * rs, rs

        def tok_ok(tok):
            return jnp.broadcast_to(tok[0:8], (8, 128)) > -1.0

        ln_tok = []
        def ln1(i):
            for r in range(TM // 16):
                r0 = i * TM + r * 16
                xb = x_v[r0:r0 + 16, :]
                if LNCH1 and len(ln_tok) >= LNCH1:
                    xb = or_gate(xb, jnp.where(tok_ok(ln_tok[-LNCH1]), 0, 1).astype(i32))
                n, rs = ln_norm(xb.astype(f32))
                ln_tok.append(rs)
                h_v[r0:r0 + 16, :] = (n * two(mod_v[:, D:2 * D]) + two(mod_v[:, 0:D])).astype(bf16)

        def ln1_stats(i):
            for r in range(TM // 16):
                r0 = i * TM + r * 16
                n, _ = ln_norm(x_v[r0:r0 + 16, :].astype(f32))
                for c in range(8):
                    qS[c, r0:r0 + 16, :] = n[:, c * 128:(c + 1) * 128]

        def ln1_half(i, ks):
            r0 = i * TM
            for c in range(ks.start // 128, ks.stop // 128):
                cs = slice(c * 128, (c + 1) * 128)
                s1 = jnp.concatenate([mod_v[:, D + c * 128:D + (c + 1) * 128]] * (TM // 8), axis=0)
                sh = jnp.concatenate([mod_v[:, c * 128:(c + 1) * 128]] * (TM // 8), axis=0)
                h_v[r0:r0 + TM, cs] = (qS[c, r0:r0 + TM, :] * s1 + sh).astype(bf16)

        def ln2(i):
            tok = []
            for r in range(TM // 16):
                r0 = i * TM + r * 16
                if not isinstance(r0, int): r0 = pl.multiple_of(r0, 16)
                x = x1_v[pl.ds(r0, 16), :]
                if LNCH and len(tok) >= LNCH:
                    gz = jnp.where(tok_ok(tok[-LNCH]), 0.0, 1.0)
                    x = x + two(jnp.concatenate([gz] * 8, axis=1))
                n, rs = ln_norm(x)
                h_v[pl.ds(r0, 16), :] = (n * two(mod_v[:, 4 * D:5 * D]) + two(mod_v[:, 3 * D:4 * D])).astype(bf16)
                tok.append(rs)
            return tok

        def proj(i, t, dst, pad, ks=None, add=False, gate=None):
            r0 = i * TM
            ks = ks or slice(0, D)
            h = h_v[r0:r0 + TM, ks]
            if gate is not None: h = or_gate(h, gate)
            r = lax.dot_general(h, wp_v[t * D:(t + 1) * D, ks], NT, preferred_element_type=f32)
            for c in range(8):
                rr = r[:, c * 128:(c + 1) * 128]
                if add: rr = rr + dst[c, pad + r0:pad + r0 + TM, :]
                dst[c, pad + r0:pad + r0 + TM, :] = rr

        def proj_mod(i, t, dst, pad, sc, tiles):
            r0 = i * TM
            h = h_v[r0:r0 + TM, :]
            for c in range(8):
                wt = wp_v[t * D + c * 128:t * D + (c + 1) * 128, :]
                j = tiles[c]
                hk = D // 2
                r = lax.dot_general(h[:, :hk], wt[:, :hk], NT, preferred_element_type=f32)
                m = jnp.dot(sc[:, :hk], wmod_v[0:hk, j * 128:(j + 1) * 128], preferred_element_type=f32)
                r = r + lax.dot_general(h[:, hk:], wt[:, hk:], NT, preferred_element_type=f32)
                m = m + jnp.dot(sc[:, hk:], wmod_v[hk:, j * 128:(j + 1) * 128], preferred_element_type=f32)
                dst[c, pad + r0:pad + r0 + TM, :] = r
                m = m[0:8]
                if 4 * 8 <= j < 5 * 8: m = m + 1.0
                mod_v[:, j * 128:(j + 1) * 128] = m

        lane = lax.broadcasted_iota(i32, (R, 128), 1)
        ix1, ix2 = lane ^ 1, lane ^ 2
        chain = []
        def att(i):
            ch = CHL if (CHL and NB - 1 - NCL <= i < NB - 1) else CHAIN
            for r in range(TM // R):
                r0 = i * TM + r * R
                qs = QSCALE
                if ch and len(chain) >= ch:
                    qs = jnp.where(chain[-ch] > -1.0, QSCALE, QSCALE * (1 + 2.0 ** -20))
                q = [qS[c, r0:r0 + R, :] * qs for c in range(8)]
                lg = []
                for w in range(W):
                    b0 = PAD + r0 - DIL * w
                    p = q[0] * kS[0, b0:b0 + R, :]
                    for c in range(1, 8):
                        p = p + q[c] * kS[c, b0:b0 + R, :]
                    p = p + jnp.take_along_axis(p, ix1, axis=1)
                    p = p + jnp.take_along_axis(p, ix2, axis=1)
                    if r0 < DIL * w:
                        row = lax.broadcasted_iota(i32, (R, 128), 0) + r0
                        p = jnp.where(row >= DIL * w, p, NEG)
                    lg.append(p)
                mx = jnp.maximum
                m = mx(mx(mx(lg[0], lg[1]), mx(lg[2], lg[3])), mx(mx(lg[4], lg[5]), mx(lg[6], lg[7])))
                e = [jnp.exp2(l - m) for l in lg]
                den = ((e[0] + e[1]) + (e[2] + e[3])) + ((e[4] + e[5]) + (e[6] + e[7]))
                inv = 1.0 / den
                chain.append(e[0])
                for c in range(8):
                    o = e[0] * vS[c, PAD + r0:PAD + r0 + R, :]
                    for w in range(1, W):
                        b0 = PAD + r0 - DIL * w
                        o = o + e[w] * vS[c, b0:b0 + R, :]
                    oS[r0:r0 + R, c * 128:(c + 1) * 128] = (o * inv).astype(bf16)

        def wo_mm(i):
            r0 = i * TM
            a = jnp.dot(oS[r0:r0 + TM, :], wop_v[...], preferred_element_type=f32)
            ga = mod_v[:, 2 * D:3 * D]
            x1_v[r0:r0 + TM, :] = x_v[r0:r0 + TM, :].astype(f32) + jnp.concatenate([ga] * (TM // 8), axis=0) * a

        def ffn_part(rows, chunks, mid=None):
            h = h_v[rows, :]
            acc = None
            for n, f in enumerate(chunks):
                if mid is not None and n == mid[0]:
                    mid[1]()
                fs = slice(f * TF, (f + 1) * TF)
                g = jnp.dot(h, w1_v[:, fs], preferred_element_type=f32)
                u = jnp.dot(h, w3_v[:, fs], preferred_element_type=f32)
                a = (g * jax.nn.sigmoid(g) * u).astype(bf16)
                y = jnp.dot(a, w2_v[fs, :], preferred_element_type=f32)
                acc = y if acc is None else acc + y
            return acc

        def mod_half(sc, dmas, ks):
            for d in dmas: d.wait()
            for o in (D, 0):
                r = jnp.dot(sc, wmod_v[:, o + ks.start:o + ks.stop], preferred_element_type=f32)[0:8]
                mod_v[:, o + ks.start:o + ks.stop] = r + 1.0 if o == D else r

        with scope('w_xa'):
            d_xa.wait()
        with scope('stats'):
            for i in range(NS): ln1_stats(i)
        with scope('w_wva'):
            d_wv[0].wait()
        with scope('prep_va'):
            prep_w(2, KQ[0])
        d_c.wait()
        cf = c_v[...].astype(f32)
        sc = jnp.broadcast_to((cf * jax.nn.sigmoid(cf)).astype(bf16), (16, D))
        for j in range(KSP):
            with scope(f'mod{j}'):
                mod_half(sc, d_m[j], KQ[j])
                if j == KSP - 1: d_xn.wait()
            with scope(f'RV{j}'):
                ln1_half(0, KQ[j])
                proj(0, 2, vS, PAD, KQ[j], add=j > 0)
                if j + 1 < KSP:
                    d_wv[j + 1].wait()
                    prep_w(2, KQ[j + 1])
                for i in range(1, NS):
                    ln1_half(i, KQ[j])
                    proj(i, 2, vS, PAD, KQ[j], add=j > 0)
                if j == KSP - 1: ln1(NS)
        with scope('w_xb'):
            d_xb.wait()
        with scope('R3'):
            for i in range(NS + 1, NS + NV1 + 1): ln1(i)
            for i in range(NS, NS + NV1): proj(i, 2, vS, PAD)
            d_wk.wait()
            if EARLYPREP: d_wq.wait(); d_wo.wait()
            for i in range(NS + NV1 + 1, NB): ln1(i)
            prep_w(1)
            if EARLYPREP: prep_w(0); prep_wo()
            for i in range(NS + NV1, NB): proj(i, 2, vS, PAD)
            for i in range(KL): proj(i, 1, kS, PAD)
        with scope('w_wq_wo_wmb'):
            if not EARLYPREP: d_wq.wait(); d_wo.wait()
            d_wmb.wait()

        def mod_vpu():
            scT_v[...] = jnp.broadcast_to(sc[0:1].astype(f32), (128, D)).T
            toks = []
            for j in range(16, 48):
                wb = wmod_v[:, j * 128:(j + 1) * 128]
                if MODCHN and len(toks) >= MODCHN:
                    t = toks[-MODCHN]
                    wb = or_gate(wb, jnp.where(t == t, 0, 1).astype(i32))
                pr = wb.astype(f32) * scT_v[...]
                a8 = jnp.sum(pr.reshape(D // 8, 8, 128), axis=0)
                toks.append(a8)
                m = jnp.broadcast_to(jnp.sum(a8, axis=0, keepdims=True), (8, 128))
                if 4 * 8 <= j < 5 * 8: m = m + 1.0
                mod_v[:, j * 128:(j + 1) * 128] = m

        def projm(i, t, dst, pad, tiles):
            if MODV: proj(i, t, dst, pad)
            else: proj_mod(i, t, dst, pad, sc, tiles)
        with scope('R4'):
            if not EARLYPREP:
                pw = prep_wo()
                prep_w(0, gate=nan_gate(pw) if TIE_WO else None)
            if MODV: mod_vpu()
            projm(KL, 1, kS, PAD, range(16, 24))
            projm(0, 0, qS, 0, range(24, 32))
            ltok = None
            for i in range(1, NB):
                if i == 1:
                    projm(1 + KL, 1, kS, PAD, range(32, 40))
                    projm(1, 0, qS, 0, range(40, 48))
                else:
                    if i + KL < NB:
                        gate = None
                        if TIE_LN and i + KL == TIE_LN:
                            ok = functools.reduce(jnp.logical_and, [tok_ok(t) for t in ltok[-max(LNCH, 1):]])
                            gate = jnp.where(ok, 0, 1).astype(i32)
                        proj(i + KL, 1, kS, PAD, gate=gate)
                    proj(i, 0, qS, 0)
                att(i - 1)
                wo_mm(i - 1)
                if i == 1: ltok = ln2(0)
        with scope('w_ffn'):
            if NOFFNDMA: d_w1.start(); d_w3.start(); d_w2.start()
            d_w1.wait(); d_w3.wait(); d_w2.wait()
        NC = F // TF
        with scope('R5'):
            att(NB - 1)
            ln2(1)
            acc = ffn_part(slice(0, TM), range(0, NA), mid=(NA // 2, lambda: wo_mm(NB - 1)))
            gbt = jnp.concatenate([mod_v[:, 5 * D:6 * D]] * (TM // 8), axis=0)
            x1_v[0:TM, :] = x1_v[0:TM, :] + gbt * acc

        def loopA(i, carry):
            rows = pl.ds(pl.multiple_of(i * TM, TM), TM)
            acc = ffn_part(rows, range(0, NA))
            ln2(jnp.minimum(i + 1, NB - 1))
            gbt = jnp.concatenate([mod_v[:, 5 * D:6 * D]] * (TM // 8), axis=0)
            x1_v[rows, :] = x1_v[rows, :] + gbt * acc
            return carry
        with scope('loopA'):
            lax.fori_loop(1, NB, loopA, 0)

        def loopB(i, carry):
            rows = pl.ds(pl.multiple_of(i * TM, TM), TM)
            acc = ffn_part(rows, range(NA, NC))
            gbt = jnp.concatenate([mod_v[:, 5 * D:6 * D]] * (TM // 8), axis=0)
            out_v[rows, :] = (x1_v[rows, :] + gbt * acc).astype(bf16)
            pltpu.make_async_copy(out_v.at[rows, :], out_hbm.at[rows, :], osems.at[i]).start()
            return carry
        with scope('loopB'):
            lax.fori_loop(0, NB, loopB, 0)
        with scope('tail'):
            for i in range(NB):
                rows = pl.ds(i * TM, TM)
                pltpu.make_async_copy(out_v.at[rows, :], out_hbm.at[rows, :], osems.at[i]).wait()

    V = pltpu.VMEM
    scratch = [V((S, D), bf16), V((D, 3 * D), bf16), V((3 * D, D), bf16), V((D, D), bf16), V((D, D), bf16),
               V((D, F), bf16), V((D, F), bf16), V((F, D), bf16), V((1, D), bf16), V((D, 6 * D), bf16),
               V((8, PAD + S, 128), f32), V((8, PAD + S, 128), f32), V((8, S, 128), f32), V((S, D), bf16),
               V((S, D), f32), V((S, D), bf16), V((S, D), bf16), V((8, 6 * D), f32), V((D, 128), f32),
               pltpu.SemaphoreType.DMA((11 + 3 * KSP,)), pltpu.SemaphoreType.DMA((NB,))]
    call = pl.pallas_call(kern, out_shape=jax.ShapeDtypeStruct((S, D), bf16),
                          in_specs=[pl.BlockSpec(memory_space=pl.ANY)] * 8, out_specs=pl.BlockSpec(memory_space=pl.ANY),
                          scratch_shapes=scratch,
                          compiler_params=pltpu.CompilerParams(vmem_limit_bytes=120 * 1024 * 1024))

    def fn(A_x, A_wqkv, A_wo, B_x, B_w1, B_w3, B_w2, c, w_mod):
        return call(A_x.reshape(S, D), A_wqkv, A_wo, B_w1, B_w3, B_w2, c, w_mod).reshape(1, S, D)
    return fn


_KERNEL = make()


@jax.jit
def pallas_adaLN_cond__sliding_local_dilated__glu_gated_swiglu__prompt_kernel(
    A_x, A_wqkv, A_wo, B_x, B_w1, B_w3, B_w2, c, w_mod
):
    return _KERNEL(A_x, A_wqkv, A_wo, B_x, B_w1, B_w3, B_w2, c, w_mod)
```

```python
import functools, math, contextlib
import jax, jax.numpy as jnp
from jax import lax
from jax.experimental import pallas as pl
from jax.experimental.pallas import tpu as pltpu

S, D, F, H, Dh, W, DIL = 2048, 1024, 3584, 32, 32, 8, 2
PAD = 16
bf16, f32, i32 = jnp.bfloat16, jnp.float32, jnp.int32
QSCALE = Dh ** -0.5 * math.log2(math.e)
NEG = -1e9 * math.log2(math.e)
NT = (((1,), (1,)), ((), ()))
NANBITS = 0x7FC17FC1


def make(TM=256, R=8, TF=512, CHAIN=3, LNCH=2, LNCH1=0, SCOPES=False, NA=4, MODI=2, NS=3,
         TIE_WO=0, TIE_LN=0, TIE_PK=0, KSP=4, NV1=3, EARLYPREP=1, MODV=0, MODCHN=1, PCH=0, TIEP=2, PAIR=1, FLAGS=('XLA_TPU_EVENLY_DISTRIBUTE_CRITICAL_NODES',), KL=2, CHL=None, NCL=2, NOFFNDMA=0):
    NB = S // TM
    scope = (lambda n: jax.named_scope(n)) if SCOPES else (lambda n: contextlib.nullcontext())

    def kern(x_hbm, wqkv_hbm, wo_hbm, w1_hbm, w3_hbm, w2_hbm, c_hbm, wmod_hbm, out_hbm,
             x_v, wqkv_v, wp_v, wo_v, wop_v, w1_v, w3_v, w2_v, c_v, wmod_v, kS, vS, qS, oS, x1_v, h_v, out_v, mod_v, scT_v,
             sems, osems):
        cnt = [0]
        def cp(src, dst):
            cnt[0] += 1
            return pltpu.make_async_copy(src, dst, sems.at[cnt[0] - 1])
        def cp2(src, dst, idx):
            return cp(src.at[idx], dst.at[idx])
        KQ = [slice(j * D // KSP, (j + 1) * D // KSP) for j in range(KSP)]
        d_c = cp(c_hbm, c_v)
        d_xa = cp2(x_hbm, x_v, (slice(0, NS * TM), slice(None)))
        d_wv = [cp2(wqkv_hbm, wqkv_v, (ks, slice(2 * D, 3 * D))) for ks in KQ]
        d_m = [[cp2(wmod_hbm, wmod_v, (slice(None), slice(o + ks.start, o + ks.stop))) for o in (D, 0)] for ks in KQ]
        d_xn = cp2(x_hbm, x_v, (slice(NS * TM, (NS + 1) * TM), slice(None)))
        d_xb = cp2(x_hbm, x_v, (slice((NS + 1) * TM, S), slice(None)))
        d_wk = cp2(wqkv_hbm, wqkv_v, (slice(None), slice(D, 2 * D)))
        d_wq = cp2(wqkv_hbm, wqkv_v, (slice(None), slice(0, D)))
        d_wo = cp(wo_hbm, wo_v)
        d_wmb = cp2(wmod_hbm, wmod_v, (slice(None), slice(2 * D, 6 * D)))
        d_w1 = cp(w1_hbm, w1_v)
        d_w3 = cp(w3_hbm, w3_v)
        d_w2 = cp(w2_hbm, w2_v)
        first = [d_c, d_xa]
        for j in range(KSP): first += [d_wv[j]] + d_m[j]
        for d in first + [d_xn, d_xb, d_wk, d_wq, d_wo, d_wmb] + ([] if NOFFNDMA else [d_w1, d_w3, d_w2]):
            d.start()
        kS[:, 0:PAD, :] = jnp.zeros((8, PAD, 128), f32)
        vS[:, 0:PAD, :] = jnp.zeros((8, PAD, 128), f32)

        def nan_gate(vals):
            ok = None
            for v in vals:
                t = pltpu.bitcast(v[0:16, 0:128], i32) != NANBITS
                ok = t if ok is None else jnp.logical_and(ok, t)
            return jnp.where(ok, 0, 1).astype(i32)

        def or_gate(vb, g):
            n, m = vb.shape[0] // 16, vb.shape[1] // 128
            gg = jnp.concatenate([g] * m, axis=1) if m > 1 else g
            gg = jnp.concatenate([gg] * n, axis=0) if n > 1 else gg
            return pltpu.bitcast(pltpu.bitcast(vb, i32) | gg, bf16)

        ptok = []
        def prep_w(t, ks=slice(0, D), gate=None, chained=False):
            out = []
            for g in range(8):
                col = t * D + g * 128
                wb = wqkv_v[ks, col:col + 128]
                if chained and len(ptok) >= PCH: wb = or_gate(wb, nan_gate([ptok[-PCH]]))
                wt = wb.T
                for c in range(8):
                    piece = jnp.concatenate([wt[32 * a + 4 * c:32 * a + 4 * c + 4, :] for a in range(4)], axis=0)
                    if gate is not None and g == 7 and c == 7:
                        piece = or_gate(piece, gate)
                    r0 = t * D + c * 128 + g * 16
                    wp_v[r0:r0 + 16, ks] = piece
                    out.append(piece)
                if chained: ptok.append(piece)
            return out

        def prep_wo(chained=False):
            out = []
            for g in range(8):
                wt = wo_v[g * 128:(g + 1) * 128, :]
                if chained and len(ptok) >= PCH: wt = or_gate(wt, nan_gate([ptok[-PCH]]))
                for c in range(8):
                    piece = jnp.concatenate([wt[32 * a + 4 * c:32 * a + 4 * c + 4, :] for a in range(4)], axis=0)
                    wop_v[c * 128 + g * 16:c * 128 + g * 16 + 16, :] = piece
                    out.append(piece)
                if chained: ptok.append(piece)
            return out

        def two(v):
            return jnp.concatenate([v, v], axis=0)

        def ln_norm(x):
            m = jnp.sum(x, axis=-1, keepdims=True) * (1.0 / D)
            xc = x - m
            v = jnp.sum(xc * xc, axis=-1, keepdims=True) * (1.0 / D)
            rs = lax.rsqrt(v + 1e-5)
            return xc * rs, rs

        def tok_ok(tok):
            return jnp.broadcast_to(tok[0:8], (8, 128)) > -1.0

        ln_tok = []
        def ln1(i):
            for r in range(TM // 16):
                r0 = i * TM + r * 16
                xb = x_v[r0:r0 + 16, :]
                if LNCH1 and len(ln_tok) >= LNCH1:
                    xb = or_gate(xb, jnp.where(tok_ok(ln_tok[-LNCH1]), 0, 1).astype(i32))
                n, rs = ln_norm(xb.astype(f32))
                ln_tok.append(rs)
                h_v[r0:r0 + 16, :] = (n * two(mod_v[:, D:2 * D]) + two(mod_v[:, 0:D])).astype(bf16)

        def ln1_stats(i):
            for r in range(TM // 16):
                r0 = i * TM + r * 16
                n, _ = ln_norm(x_v[r0:r0 + 16, :].astype(f32))
                for c in range(8):
                    qS[c, r0:r0 + 16, :] = n[:, c * 128:(c + 1) * 128]

        def ln1_half(i, ks):
            r0 = i * TM
            for c in range(ks.start // 128, ks.stop // 128):
                cs = slice(c * 128, (c + 1) * 128)
                s1 = jnp.concatenate([mod_v[:, D + c * 128:D + (c + 1) * 128]] * (TM // 8), axis=0)
                sh = jnp.concatenate([mod_v[:, c * 128:(c + 1) * 128]] * (TM // 8), axis=0)
                h_v[r0:r0 + TM, cs] = (qS[c, r0:r0 + TM, :] * s1 + sh).astype(bf16)

        def ln2(i):
            tok = []
            for r in range(TM // 16):
                r0 = i * TM + r * 16
                if not isinstance(r0, int): r0 = pl.multiple_of(r0, 16)
                x = x1_v[pl.ds(r0, 16), :]
                if LNCH and len(tok) >= LNCH:
                    gz = jnp.where(tok_ok(tok[-LNCH]), 0.0, 1.0)
                    x = x + two(jnp.concatenate([gz] * 8, axis=1))
                n, rs = ln_norm(x)
                h_v[pl.ds(r0, 16), :] = (n * two(mod_v[:, 4 * D:5 * D]) + two(mod_v[:, 3 * D:4 * D])).astype(bf16)
                tok.append(rs)
            return tok

        def proj(i, t, dst, pad, ks=None, add=False, gate=None):
            r0 = i * TM
            ks = ks or slice(0, D)
            h = h_v[r0:r0 + TM, ks]
            if gate is not None: h = or_gate(h, gate)
            r = lax.dot_general(h, wp_v[t * D:(t + 1) * D, ks], NT, preferred_element_type=f32)
            for c in range(8):
                rr = r[:, c * 128:(c + 1) * 128]
                if add: rr = rr + dst[c, pad + r0:pad + r0 + TM, :]
                dst[c, pad + r0:pad + r0 + TM, :] = rr

        def proj_mod(i, t, dst, pad, sc, tiles):
            r0 = i * TM
            h = h_v[r0:r0 + TM, :]
            for c in range(8):
                wt = wp_v[t * D + c * 128:t * D + (c + 1) * 128, :]
                j = tiles[c]
                hk = D // 2
                r = lax.dot_general(h[:, :hk], wt[:, :hk], NT, preferred_element_type=f32)
                m = jnp.dot(sc[:, :hk], wmod_v[0:hk, j * 128:(j + 1) * 128], preferred_element_type=f32)
                r = r + lax.dot_general(h[:, hk:], wt[:, hk:], NT, preferred_element_type=f32)
                m = m + jnp.dot(sc[:, hk:], wmod_v[hk:, j * 128:(j + 1) * 128], preferred_element_type=f32)
                dst[c, pad + r0:pad + r0 + TM, :] = r
                m = m[0:8]
                if 4 * 8 <= j < 5 * 8: m = m + 1.0
                mod_v[:, j * 128:(j + 1) * 128] = m

        lane = lax.broadcasted_iota(i32, (R, 128), 1)
        ix1, ix2 = lane ^ 1, lane ^ 2
        chain = []
        held = []
        def att(i):
            ch = CHL if (CHL and NB - 1 - NCL <= i < NB - 1) else CHAIN
            for r in range(TM // R):
                r0 = i * TM + r * R
                qs = QSCALE
                if ch and len(chain) >= ch:
                    qs = jnp.where(chain[-ch] > -1.0, QSCALE, QSCALE * (1 + 2.0 ** -20))
                q = [qS[c, r0:r0 + R, :] * qs for c in range(8)]
                lg = []
                for w in range(W):
                    b0 = PAD + r0 - DIL * w
                    p = q[0] * kS[0, b0:b0 + R, :]
                    for c in range(1, 8):
                        p = p + q[c] * kS[c, b0:b0 + R, :]
                    p = p + jnp.take_along_axis(p, ix1, axis=1)
                    p = p + jnp.take_along_axis(p, ix2, axis=1)
                    if r0 < DIL * w:
                        row = lax.broadcasted_iota(i32, (R, 128), 0) + r0
                        p = jnp.where(row >= DIL * w, p, NEG)
                    lg.append(p)
                mx = jnp.maximum
                m = mx(mx(mx(lg[0], lg[1]), mx(lg[2], lg[3])), mx(mx(lg[4], lg[5]), mx(lg[6], lg[7])))
                e = [jnp.exp2(l - m) for l in lg]
                den = ((e[0] + e[1]) + (e[2] + e[3])) + ((e[4] + e[5]) + (e[6] + e[7]))
                inv = 1.0 / den
                chain.append(e[0])
                for c in range(8):
                    o = e[0] * vS[c, PAD + r0:PAD + r0 + R, :]
                    for w in range(1, W):
                        b0 = PAD + r0 - DIL * w
                        o = o + e[w] * vS[c, b0:b0 + R, :]
                    o = o * inv
                    if PAIR and R == 8:
                        if r % 2 == 0: held.append(o)
                        else: oS[r0 - R:r0 + R, c * 128:(c + 1) * 128] = jnp.concatenate([held.pop(0), o], axis=0).astype(bf16)
                    else:
                        oS[r0:r0 + R, c * 128:(c + 1) * 128] = o.astype(bf16)

        def wo_mm(i):
            r0 = i * TM
            a = jnp.dot(oS[r0:r0 + TM, :], wop_v[...], preferred_element_type=f32)
            ga = mod_v[:, 2 * D:3 * D]
            x1_v[r0:r0 + TM, :] = x_v[r0:r0 + TM, :].astype(f32) + jnp.concatenate([ga] * (TM // 8), axis=0) * a

        def ffn_part(rows, chunks, mid=None):
            h = h_v[rows, :]
            acc = None
            for n, f in enumerate(chunks):
                if mid is not None and n == mid[0]:
                    mid[1]()
                fs = slice(f * TF, (f + 1) * TF)
                g = jnp.dot(h, w1_v[:, fs], preferred_element_type=f32)
                u = jnp.dot(h, w3_v[:, fs], preferred_element_type=f32)
                a = (g * jax.nn.sigmoid(g) * u).astype(bf16)
                y = jnp.dot(a, w2_v[fs, :], preferred_element_type=f32)
                acc = y if acc is None else acc + y
            return acc

        def mod_half(sc, dmas, ks):
            for d in dmas: d.wait()
            for o in (D, 0):
                r = jnp.dot(sc, wmod_v[:, o + ks.start:o + ks.stop], preferred_element_type=f32)[0:8]
                mod_v[:, o + ks.start:o + ks.stop] = r + 1.0 if o == D else r

        with scope('w_xa'):
            d_xa.wait()
        with scope('stats'):
            for i in range(NS): ln1_stats(i)
        with scope('w_wva'):
            d_wv[0].wait()
        with scope('prep_va'):
            prep_w(2, KQ[0])
        d_c.wait()
        cf = c_v[...].astype(f32)
        sc = jnp.broadcast_to((cf * jax.nn.sigmoid(cf)).astype(bf16), (16, D))
        for j in range(KSP):
            with scope(f'mod{j}'):
                mod_half(sc, d_m[j], KQ[j])
                if j == KSP - 1: d_xn.wait()
            with scope(f'RV{j}'):
                ln1_half(0, KQ[j])
                proj(0, 2, vS, PAD, KQ[j], add=j > 0)
                if j + 1 < KSP:
                    d_wv[j + 1].wait()
                    prep_w(2, KQ[j + 1])
                for i in range(1, NS):
                    ln1_half(i, KQ[j])
                    proj(i, 2, vS, PAD, KQ[j], add=j > 0)
                if j == KSP - 1: ln1(NS)
        with scope('w_xb'):
            d_xb.wait()
        with scope('R3'):
            for i in range(NS + 1, NS + NV1 + 1): ln1(i)
            for i in range(NS, NS + NV1): proj(i, 2, vS, PAD)
            d_wk.wait()
            if EARLYPREP: d_wq.wait(); d_wo.wait()
            for i in range(NS + NV1 + 1, NB): ln1(i)
            prep_w(1, chained=PCH > 0)
            if EARLYPREP: pq = prep_w(0, chained=PCH > 0); pw = prep_wo(chained=PCH > 0)
            for i in range(NS + NV1, NB): proj(i, 2, vS, PAD)
            for i in range(KL):
                gate = None
                if EARLYPREP and TIEP == 1 and i == KL - 1: gate = nan_gate(pw[-8:])
                if EARLYPREP and TIEP == 2: gate = nan_gate(pq if i == 0 else pw)
                proj(i, 1, kS, PAD, gate=gate)
        with scope('w_wq_wo_wmb'):
            if not EARLYPREP: d_wq.wait(); d_wo.wait()
            d_wmb.wait()

        def mod_vpu():
            scT_v[...] = jnp.broadcast_to(sc[0:1].astype(f32), (128, D)).T
            toks = []
            for j in range(16, 48):
                wb = wmod_v[:, j * 128:(j + 1) * 128]
                if MODCHN and len(toks) >= MODCHN:
                    t = toks[-MODCHN]
                    wb = or_gate(wb, jnp.where(t == t, 0, 1).astype(i32))
                pr = wb.astype(f32) * scT_v[...]
                a8 = jnp.sum(pr.reshape(D // 8, 8, 128), axis=0)
                toks.append(a8)
                m = jnp.broadcast_to(jnp.sum(a8, axis=0, keepdims=True), (8, 128))
                if 4 * 8 <= j < 5 * 8: m = m + 1.0
                mod_v[:, j * 128:(j + 1) * 128] = m

        def projm(i, t, dst, pad, tiles):
            if MODV: proj(i, t, dst, pad)
            else: proj_mod(i, t, dst, pad, sc, tiles)
        with scope('R4'):
            if not EARLYPREP:
                pw = prep_wo()
                prep_w(0, gate=nan_gate(pw) if TIE_WO else None)
            if MODV: mod_vpu()
            projm(KL, 1, kS, PAD, range(16, 24))
            projm(0, 0, qS, 0, range(24, 32))
            ltok = None
            for i in range(1, NB):
                if i == 1:
                    projm(1 + KL, 1, kS, PAD, range(32, 40))
                    projm(1, 0, qS, 0, range(40, 48))
                else:
                    if i + KL < NB:
                        gate = None
                        if TIE_LN and i + KL == TIE_LN:
                            ok = functools.reduce(jnp.logical_and, [tok_ok(t) for t in ltok[-max(LNCH, 1):]])
                            gate = jnp.where(ok, 0, 1).astype(i32)
                        proj(i + KL, 1, kS, PAD, gate=gate)
                    proj(i, 0, qS, 0)
                att(i - 1)
                wo_mm(i - 1)
                if i == 1: ltok = ln2(0)
        with scope('w_ffn'):
            if NOFFNDMA: d_w1.start(); d_w3.start(); d_w2.start()
            d_w1.wait(); d_w3.wait(); d_w2.wait()
        NC = F // TF
        with scope('R5'):
            att(NB - 1)
            ln2(1)
            acc = ffn_part(slice(0, TM), range(0, NA), mid=(NA // 2, lambda: wo_mm(NB - 1)))
            gbt = jnp.concatenate([mod_v[:, 5 * D:6 * D]] * (TM // 8), axis=0)
            x1_v[0:TM, :] = x1_v[0:TM, :] + gbt * acc

        def loopA(i, carry):
            rows = pl.ds(pl.multiple_of(i * TM, TM), TM)
            acc = ffn_part(rows, range(0, NA))
            ln2(jnp.minimum(i + 1, NB - 1))
            gbt = jnp.concatenate([mod_v[:, 5 * D:6 * D]] * (TM // 8), axis=0)
            x1_v[rows, :] = x1_v[rows, :] + gbt * acc
            return carry
        with scope('loopA'):
            lax.fori_loop(1, NB, loopA, 0)

        def loopB(i, carry):
            rows = pl.ds(pl.multiple_of(i * TM, TM), TM)
            acc = ffn_part(rows, range(NA, NC))
            gbt = jnp.concatenate([mod_v[:, 5 * D:6 * D]] * (TM // 8), axis=0)
            out_v[rows, :] = (x1_v[rows, :] + gbt * acc).astype(bf16)
            pltpu.make_async_copy(out_v.at[rows, :], out_hbm.at[rows, :], osems.at[i]).start()
            return carry
        with scope('loopB'):
            lax.fori_loop(0, NB, loopB, 0)
        with scope('tail'):
            for i in range(NB):
                rows = pl.ds(i * TM, TM)
                pltpu.make_async_copy(out_v.at[rows, :], out_hbm.at[rows, :], osems.at[i]).wait()

    V = pltpu.VMEM
    scratch = [V((S, D), bf16), V((D, 3 * D), bf16), V((3 * D, D), bf16), V((D, D), bf16), V((D, D), bf16),
               V((D, F), bf16), V((D, F), bf16), V((F, D), bf16), V((1, D), bf16), V((D, 6 * D), bf16),
               V((8, PAD + S, 128), f32), V((8, PAD + S, 128), f32), V((8, S, 128), f32), V((S, D), bf16),
               V((S, D), f32), V((S, D), bf16), V((S, D), bf16), V((8, 6 * D), f32), V((D, 128), f32),
               pltpu.SemaphoreType.DMA((11 + 3 * KSP,)), pltpu.SemaphoreType.DMA((NB,))]
    call = pl.pallas_call(kern, out_shape=jax.ShapeDtypeStruct((S, D), bf16),
                          in_specs=[pl.BlockSpec(memory_space=pl.ANY)] * 8, out_specs=pl.BlockSpec(memory_space=pl.ANY),
                          scratch_shapes=scratch,
                          compiler_params=pltpu.CompilerParams(vmem_limit_bytes=120 * 1024 * 1024, flags={f: True for f in FLAGS} or None))

    def fn(A_x, A_wqkv, A_wo, B_x, B_w1, B_w3, B_w2, c, w_mod):
        return call(A_x.reshape(S, D), A_wqkv, A_wo, B_w1, B_w3, B_w2, c, w_mod).reshape(1, S, D)
    return fn


_KERNEL = make()


@jax.jit
def pallas_adaLN_cond__sliding_local_dilated__glu_gated_swiglu__prompt_kernel(
    A_x, A_wqkv, A_wo, B_x, B_w1, B_w3, B_w2, c, w_mod
):
    return _KERNEL(A_x, A_wqkv, A_wo, B_x, B_w1, B_w3, B_w2, c, w_mod)
```

```python
import functools, math, contextlib
import jax, jax.numpy as jnp
from jax import lax
from jax.experimental import pallas as pl
from jax.experimental.pallas import tpu as pltpu

S, D, F, H, Dh, W, DIL = 2048, 1024, 3584, 32, 32, 8, 2
PAD = 16
bf16, f32, i32 = jnp.bfloat16, jnp.float32, jnp.int32
QSCALE = Dh ** -0.5 * math.log2(math.e)
NEG = -1e9 * math.log2(math.e)
NT = (((1,), (1,)), ((), ()))
NANBITS = 0x7FC17FC1


def make(TM=256, R=8, TF=512, CHAIN=3, LNCH=2, LNCH1=0, SCOPES=False, NA=4, MODI=2, NS=3,
         TIE_WO=0, TIE_LN=0, TIE_PK=0, KSP=4, NV1=3, EARLYPREP=1, MODV=1, MODCHN=0, PCH=0, TIEP=2, PAIR=1, FLAGS=('XLA_TPU_EVENLY_DISTRIBUTE_CRITICAL_NODES',), KL=2, CHL=None, NCL=2, NOFFNDMA=0):
    NB = S // TM
    scope = (lambda n: jax.named_scope(n)) if SCOPES else (lambda n: contextlib.nullcontext())

    def kern(x_hbm, wqkv_hbm, wo_hbm, w1_hbm, w3_hbm, w2_hbm, c_hbm, wmod_hbm, out_hbm,
             x_v, wqkv_v, wp_v, wo_v, wop_v, w1_v, w3_v, w2_v, c_v, wmod_v, kS, vS, qS, oS, x1_v, h_v, out_v, mod_v, scT_v,
             sems, osems):
        cnt = [0]
        def cp(src, dst):
            cnt[0] += 1
            return pltpu.make_async_copy(src, dst, sems.at[cnt[0] - 1])
        def cp2(src, dst, idx):
            return cp(src.at[idx], dst.at[idx])
        KQ = [slice(j * D // KSP, (j + 1) * D // KSP) for j in range(KSP)]
        d_c = cp(c_hbm, c_v)
        d_xa = cp2(x_hbm, x_v, (slice(0, NS * TM), slice(None)))
        d_wv = [cp2(wqkv_hbm, wqkv_v, (ks, slice(2 * D, 3 * D))) for ks in KQ]
        d_m = [[cp2(wmod_hbm, wmod_v, (slice(None), slice(o + ks.start, o + ks.stop))) for o in (D, 0)] for ks in KQ]
        d_xn = cp2(x_hbm, x_v, (slice(NS * TM, (NS + 1) * TM), slice(None)))
        d_xb = cp2(x_hbm, x_v, (slice((NS + 1) * TM, S), slice(None)))
        d_wk = cp2(wqkv_hbm, wqkv_v, (slice(None), slice(D, 2 * D)))
        d_wq = cp2(wqkv_hbm, wqkv_v, (slice(None), slice(0, D)))
        d_wo = cp(wo_hbm, wo_v)
        d_wmb = cp2(wmod_hbm, wmod_v, (slice(None), slice(2 * D, 6 * D)))
        d_w1 = cp(w1_hbm, w1_v)
        d_w3 = cp(w3_hbm, w3_v)
        d_w2 = cp(w2_hbm, w2_v)
        first = [d_c, d_xa]
        for j in range(KSP): first += [d_wv[j]] + d_m[j]
        for d in first + [d_xn, d_xb, d_wk, d_wq, d_wo, d_wmb] + ([] if NOFFNDMA else [d_w1, d_w3, d_w2]):
            d.start()
        kS[:, 0:PAD, :] = jnp.zeros((8, PAD, 128), f32)
        vS[:, 0:PAD, :] = jnp.zeros((8, PAD, 128), f32)

        def nan_gate(vals):
            ok = None
            for v in vals:
                t = pltpu.bitcast(v[0:16, 0:128], i32) != NANBITS
                ok = t if ok is None else jnp.logical_and(ok, t)
            return jnp.where(ok, 0, 1).astype(i32)

        def or_gate(vb, g):
            n, m = vb.shape[0] // 16, vb.shape[1] // 128
            gg = jnp.concatenate([g] * m, axis=1) if m > 1 else g
            gg = jnp.concatenate([gg] * n, axis=0) if n > 1 else gg
            return pltpu.bitcast(pltpu.bitcast(vb, i32) | gg, bf16)

        ptok = []
        def prep_w(t, ks=slice(0, D), gate=None, chained=False):
            out = []
            for g in range(8):
                col = t * D + g * 128
                wb = wqkv_v[ks, col:col + 128]
                if chained and len(ptok) >= PCH: wb = or_gate(wb, nan_gate([ptok[-PCH]]))
                wt = wb.T
                for c in range(8):
                    piece = jnp.concatenate([wt[32 * a + 4 * c:32 * a + 4 * c + 4, :] for a in range(4)], axis=0)
                    if gate is not None and g == 7 and c == 7:
                        piece = or_gate(piece, gate)
                    r0 = t * D + c * 128 + g * 16
                    wp_v[r0:r0 + 16, ks] = piece
                    out.append(piece)
                if chained: ptok.append(piece)
            return out

        def prep_wo(chained=False):
            out = []
            for g in range(8):
                wt = wo_v[g * 128:(g + 1) * 128, :]
                if chained and len(ptok) >= PCH: wt = or_gate(wt, nan_gate([ptok[-PCH]]))
                for c in range(8):
                    piece = jnp.concatenate([wt[32 * a + 4 * c:32 * a + 4 * c + 4, :] for a in range(4)], axis=0)
                    wop_v[c * 128 + g * 16:c * 128 + g * 16 + 16, :] = piece
                    out.append(piece)
                if chained: ptok.append(piece)
            return out

        def two(v):
            return jnp.concatenate([v, v], axis=0)

        def ln_norm(x):
            m = jnp.sum(x, axis=-1, keepdims=True) * (1.0 / D)
            xc = x - m
            v = jnp.sum(xc * xc, axis=-1, keepdims=True) * (1.0 / D)
            rs = lax.rsqrt(v + 1e-5)
            return xc * rs, rs

        def tok_ok(tok):
            return jnp.broadcast_to(tok[0:8], (8, 128)) > -1.0

        ln_tok = []
        def ln1(i):
            for r in range(TM // 16):
                r0 = i * TM + r * 16
                xb = x_v[r0:r0 + 16, :]
                if LNCH1 and len(ln_tok) >= LNCH1:
                    xb = or_gate(xb, jnp.where(tok_ok(ln_tok[-LNCH1]), 0, 1).astype(i32))
                n, rs = ln_norm(xb.astype(f32))
                ln_tok.append(rs)
                h_v[r0:r0 + 16, :] = (n * two(mod_v[:, D:2 * D]) + two(mod_v[:, 0:D])).astype(bf16)

        def ln1_stats(i):
            for r in range(TM // 16):
                r0 = i * TM + r * 16
                n, _ = ln_norm(x_v[r0:r0 + 16, :].astype(f32))
                for c in range(8):
                    qS[c, r0:r0 + 16, :] = n[:, c * 128:(c + 1) * 128]

        def ln1_half(i, ks):
            r0 = i * TM
            for c in range(ks.start // 128, ks.stop // 128):
                cs = slice(c * 128, (c + 1) * 128)
                s1 = jnp.concatenate([mod_v[:, D + c * 128:D + (c + 1) * 128]] * (TM // 8), axis=0)
                sh = jnp.concatenate([mod_v[:, c * 128:(c + 1) * 128]] * (TM // 8), axis=0)
                h_v[r0:r0 + TM, cs] = (qS[c, r0:r0 + TM, :] * s1 + sh).astype(bf16)

        def ln2(i):
            tok = []
            for r in range(TM // 16):
                r0 = i * TM + r * 16
                if not isinstance(r0, int): r0 = pl.multiple_of(r0, 16)
                x = x1_v[pl.ds(r0, 16), :]
                if LNCH and len(tok) >= LNCH:
                    gz = jnp.where(tok_ok(tok[-LNCH]), 0.0, 1.0)
                    x = x + two(jnp.concatenate([gz] * 8, axis=1))
                n, rs = ln_norm(x)
                h_v[pl.ds(r0, 16), :] = (n * two(mod_v[:, 4 * D:5 * D]) + two(mod_v[:, 3 * D:4 * D])).astype(bf16)
                tok.append(rs)
            return tok

        def proj(i, t, dst, pad, ks=None, add=False, gate=None):
            r0 = i * TM
            ks = ks or slice(0, D)
            h = h_v[r0:r0 + TM, ks]
            if gate is not None: h = or_gate(h, gate)
            r = lax.dot_general(h, wp_v[t * D:(t + 1) * D, ks], NT, preferred_element_type=f32)
            for c in range(8):
                rr = r[:, c * 128:(c + 1) * 128]
                if add: rr = rr + dst[c, pad + r0:pad + r0 + TM, :]
                dst[c, pad + r0:pad + r0 + TM, :] = rr

        def proj_mod(i, t, dst, pad, sc, tiles):
            r0 = i * TM
            h = h_v[r0:r0 + TM, :]
            for c in range(8):
                wt = wp_v[t * D + c * 128:t * D + (c + 1) * 128, :]
                j = tiles[c]
                hk = D // 2
                r = lax.dot_general(h[:, :hk], wt[:, :hk], NT, preferred_element_type=f32)
                m = jnp.dot(sc[:, :hk], wmod_v[0:hk, j * 128:(j + 1) * 128], preferred_element_type=f32)
                r = r + lax.dot_general(h[:, hk:], wt[:, hk:], NT, preferred_element_type=f32)
                m = m + jnp.dot(sc[:, hk:], wmod_v[hk:, j * 128:(j + 1) * 128], preferred_element_type=f32)
                dst[c, pad + r0:pad + r0 + TM, :] = r
                m = m[0:8]
                if 4 * 8 <= j < 5 * 8: m = m + 1.0
                mod_v[:, j * 128:(j + 1) * 128] = m

        lane = lax.broadcasted_iota(i32, (R, 128), 1)
        ix1, ix2 = lane ^ 1, lane ^ 2
        chain = []
        held = []
        def att(i):
            ch = CHL if (CHL and NB - 1 - NCL <= i < NB - 1) else CHAIN
            for r in range(TM // R):
                r0 = i * TM + r * R
                qs = QSCALE
                if ch and len(chain) >= ch:
                    qs = jnp.where(chain[-ch] > -1.0, QSCALE, QSCALE * (1 + 2.0 ** -20))
                q = [qS[c, r0:r0 + R, :] * qs for c in range(8)]
                lg = []
                for w in range(W):
                    b0 = PAD + r0 - DIL * w
                    p = q[0] * kS[0, b0:b0 + R, :]
                    for c in range(1, 8):
                        p = p + q[c] * kS[c, b0:b0 + R, :]
                    p = p + jnp.take_along_axis(p, ix1, axis=1)
                    p = p + jnp.take_along_axis(p, ix2, axis=1)
                    if r0 < DIL * w:
                        row = lax.broadcasted_iota(i32, (R, 128), 0) + r0
                        p = jnp.where(row >= DIL * w, p, NEG)
                    lg.append(p)
                mx = jnp.maximum
                m = mx(mx(mx(lg[0], lg[1]), mx(lg[2], lg[3])), mx(mx(lg[4], lg[5]), mx(lg[6], lg[7])))
                e = [jnp.exp2(l - m) for l in lg]
                den = ((e[0] + e[1]) + (e[2] + e[3])) + ((e[4] + e[5]) + (e[6] + e[7]))
                inv = 1.0 / den
                chain.append(e[0])
                for c in range(8):
                    o = e[0] * vS[c, PAD + r0:PAD + r0 + R, :]
                    for w in range(1, W):
                        b0 = PAD + r0 - DIL * w
                        o = o + e[w] * vS[c, b0:b0 + R, :]
                    o = o * inv
                    if PAIR and R == 8:
                        if r % 2 == 0: held.append(o)
                        else: oS[r0 - R:r0 + R, c * 128:(c + 1) * 128] = jnp.concatenate([held.pop(0), o], axis=0).astype(bf16)
                    else:
                        oS[r0:r0 + R, c * 128:(c + 1) * 128] = o.astype(bf16)

        def wo_mm(i):
            r0 = i * TM
            a = jnp.dot(oS[r0:r0 + TM, :], wop_v[...], preferred_element_type=f32)
            ga = mod_v[:, 2 * D:3 * D]
            x1_v[r0:r0 + TM, :] = x_v[r0:r0 + TM, :].astype(f32) + jnp.concatenate([ga] * (TM // 8), axis=0) * a

        def ffn_part(rows, chunks, mid=None):
            h = h_v[rows, :]
            acc = None
            for n, f in enumerate(chunks):
                if mid is not None and n == mid[0]:
                    mid[1]()
                fs = slice(f * TF, (f + 1) * TF)
                g = jnp.dot(h, w1_v[:, fs], preferred_element_type=f32)
                u = jnp.dot(h, w3_v[:, fs], preferred_element_type=f32)
                a = (g * jax.nn.sigmoid(g) * u).astype(bf16)
                y = jnp.dot(a, w2_v[fs, :], preferred_element_type=f32)
                acc = y if acc is None else acc + y
            return acc

        def mod_half(sc, dmas, ks):
            for d in dmas: d.wait()
            for o in (D, 0):
                r = jnp.dot(sc, wmod_v[:, o + ks.start:o + ks.stop], preferred_element_type=f32)[0:8]
                mod_v[:, o + ks.start:o + ks.stop] = r + 1.0 if o == D else r

        with scope('w_xa'):
            d_xa.wait()
        with scope('stats'):
            for i in range(NS): ln1_stats(i)
        with scope('w_wva'):
            d_wv[0].wait()
        with scope('prep_va'):
            prep_w(2, KQ[0])
        d_c.wait()
        cf = c_v[...].astype(f32)
        sc = jnp.broadcast_to((cf * jax.nn.sigmoid(cf)).astype(bf16), (16, D))
        for j in range(KSP):
            with scope(f'mod{j}'):
                mod_half(sc, d_m[j], KQ[j])
                if j == KSP - 1: d_xn.wait()
            with scope(f'RV{j}'):
                ln1_half(0, KQ[j])
                proj(0, 2, vS, PAD, KQ[j], add=j > 0)
                if j + 1 < KSP:
                    d_wv[j + 1].wait()
                    prep_w(2, KQ[j + 1])
                for i in range(1, NS):
                    ln1_half(i, KQ[j])
                    proj(i, 2, vS, PAD, KQ[j], add=j > 0)
                if j == KSP - 1: ln1(NS)
        with scope('w_xb'):
            d_xb.wait()
        with scope('R3'):
            for i in range(NS + 1, NS + NV1 + 1): ln1(i)
            for i in range(NS, NS + NV1): proj(i, 2, vS, PAD)
            d_wk.wait()
            if EARLYPREP: d_wq.wait(); d_wo.wait()
            for i in range(NS + NV1 + 1, NB): ln1(i)
            prep_w(1, chained=PCH > 0)
            if EARLYPREP: pq = prep_w(0, chained=PCH > 0); pw = prep_wo(chained=PCH > 0)
            for i in range(NS + NV1, NB): proj(i, 2, vS, PAD)
            for i in range(KL):
                gate = None
                if EARLYPREP and TIEP == 1 and i == KL - 1: gate = nan_gate(pw[-8:])
                if EARLYPREP and TIEP == 2: gate = nan_gate(pq if i == 0 else pw)
                proj(i, 1, kS, PAD, gate=gate)
        with scope('w_wq_wo_wmb'):
            if not EARLYPREP: d_wq.wait(); d_wo.wait()
            d_wmb.wait()

        def mod_vpu():
            scT_v[...] = jnp.broadcast_to(sc[0:1].astype(f32), (128, D)).T
            toks = []
            for j in range(16, 48):
                wb = wmod_v[:, j * 128:(j + 1) * 128]
                if MODCHN and len(toks) >= MODCHN:
                    t = toks[-MODCHN]
                    wb = or_gate(wb, jnp.where(t == t, 0, 1).astype(i32))
                pr = wb.astype(f32) * scT_v[...]
                a8 = jnp.sum(pr.reshape(D // 8, 8, 128), axis=0)
                toks.append(a8)
                m = jnp.broadcast_to(jnp.sum(a8, axis=0, keepdims=True), (8, 128))
                if 4 * 8 <= j < 5 * 8: m = m + 1.0
                mod_v[:, j * 128:(j + 1) * 128] = m
                mtok[j] = m

        mtok = {}
        def projm(i, t, dst, pad, tiles):
            if MODV:
                gate = None
                prev = [mtok[j - 8 * MODV] for j in tiles if j - 8 * MODV in mtok]
                if tiles[0] == 40: prev += [mtok[j] for j in range(48 - 8 * MODV, 48)] if MODV else []
                if prev:
                    ok = functools.reduce(jnp.logical_and, [m == m for m in prev])
                    gate = jnp.where(ok, 0, 1).astype(i32)
                proj(i, t, dst, pad, gate=gate)
            else: proj_mod(i, t, dst, pad, sc, tiles)
        with scope('R4'):
            if not EARLYPREP:
                pw = prep_wo()
                prep_w(0, gate=nan_gate(pw) if TIE_WO else None)
            if MODV: mod_vpu()
            projm(KL, 1, kS, PAD, range(16, 24))
            projm(0, 0, qS, 0, range(24, 32))
            ltok = None
            for i in range(1, NB):
                if i == 1:
                    projm(1 + KL, 1, kS, PAD, range(32, 40))
                    projm(1, 0, qS, 0, range(40, 48))
                else:
                    if i + KL < NB:
                        gate = None
                        if TIE_LN and i + KL == TIE_LN:
                            ok = functools.reduce(jnp.logical_and, [tok_ok(t) for t in ltok[-max(LNCH, 1):]])
                            gate = jnp.where(ok, 0, 1).astype(i32)
                        proj(i + KL, 1, kS, PAD, gate=gate)
                    proj(i, 0, qS, 0)
                att(i - 1)
                wo_mm(i - 1)
                if i == 1: ltok = ln2(0)
        with scope('w_ffn'):
            if NOFFNDMA: d_w1.start(); d_w3.start(); d_w2.start()
            d_w1.wait(); d_w3.wait(); d_w2.wait()
        NC = F // TF
        with scope('R5'):
            att(NB - 1)
            ln2(1)
            acc = ffn_part(slice(0, TM), range(0, NA), mid=(NA // 2, lambda: wo_mm(NB - 1)))
            gbt = jnp.concatenate([mod_v[:, 5 * D:6 * D]] * (TM // 8), axis=0)
            x1_v[0:TM, :] = x1_v[0:TM, :] + gbt * acc

        def loopA(i, carry):
            rows = pl.ds(pl.multiple_of(i * TM, TM), TM)
            acc = ffn_part(rows, range(0, NA))
            ln2(jnp.minimum(i + 1, NB - 1))
            gbt = jnp.concatenate([mod_v[:, 5 * D:6 * D]] * (TM // 8), axis=0)
            x1_v[rows, :] = x1_v[rows, :] + gbt * acc
            return carry
        with scope('loopA'):
            lax.fori_loop(1, NB, loopA, 0)

        def loopB(i, carry):
            rows = pl.ds(pl.multiple_of(i * TM, TM), TM)
            acc = ffn_part(rows, range(NA, NC))
            gbt = jnp.concatenate([mod_v[:, 5 * D:6 * D]] * (TM // 8), axis=0)
            out_v[rows, :] = (x1_v[rows, :] + gbt * acc).astype(bf16)
            pltpu.make_async_copy(out_v.at[rows, :], out_hbm.at[rows, :], osems.at[i]).start()
            return carry
        with scope('loopB'):
            lax.fori_loop(0, NB, loopB, 0)
        with scope('tail'):
            for i in range(NB):
                rows = pl.ds(i * TM, TM)
                pltpu.make_async_copy(out_v.at[rows, :], out_hbm.at[rows, :], osems.at[i]).wait()

    V = pltpu.VMEM
    scratch = [V((S, D), bf16), V((D, 3 * D), bf16), V((3 * D, D), bf16), V((D, D), bf16), V((D, D), bf16),
               V((D, F), bf16), V((D, F), bf16), V((F, D), bf16), V((1, D), bf16), V((D, 6 * D), bf16),
               V((8, PAD + S, 128), f32), V((8, PAD + S, 128), f32), V((8, S, 128), f32), V((S, D), bf16),
               V((S, D), f32), V((S, D), bf16), V((S, D), bf16), V((8, 6 * D), f32), V((D, 128), f32),
               pltpu.SemaphoreType.DMA((11 + 3 * KSP,)), pltpu.SemaphoreType.DMA((NB,))]
    call = pl.pallas_call(kern, out_shape=jax.ShapeDtypeStruct((S, D), bf16),
                          in_specs=[pl.BlockSpec(memory_space=pl.ANY)] * 8, out_specs=pl.BlockSpec(memory_space=pl.ANY),
                          scratch_shapes=scratch,
                          compiler_params=pltpu.CompilerParams(vmem_limit_bytes=120 * 1024 * 1024, flags={f: True for f in FLAGS} or None))

    def fn(A_x, A_wqkv, A_wo, B_x, B_w1, B_w3, B_w2, c, w_mod):
        return call(A_x.reshape(S, D), A_wqkv, A_wo, B_w1, B_w3, B_w2, c, w_mod).reshape(1, S, D)
    return fn


_KERNEL = make()


@jax.jit
def pallas_adaLN_cond__sliding_local_dilated__glu_gated_swiglu__prompt_kernel(
    A_x, A_wqkv, A_wo, B_x, B_w1, B_w3, B_w2, c, w_mod
):
    return _KERNEL(A_x, A_wqkv, A_wo, B_x, B_w1, B_w3, B_w2, c, w_mod)
```

```python
import functools, math, contextlib
import jax, jax.numpy as jnp
from jax import lax
from jax.experimental import pallas as pl
from jax.experimental.pallas import tpu as pltpu

S, D, F, H, Dh, W, DIL = 2048, 1024, 3584, 32, 32, 8, 2
PAD = 16
bf16, f32, i32 = jnp.bfloat16, jnp.float32, jnp.int32
QSCALE = Dh ** -0.5 * math.log2(math.e)
NEG = -1e9 * math.log2(math.e)
NT = (((1,), (1,)), ((), ()))
NANBITS = 0x7FC17FC1


def make(TM=256, R=8, TF=512, CHAIN=2, LNCH=2, LNCH1=0, SCOPES=False, NA=4, MODI=2, NS=3,
         TIE_WO=0, TIE_LN=0, TIE_PK=0, KSP=4, NV1=3, EARLYPREP=1, MODV=1, MODCHN=4, PCH=0, TIEP=2, PAIR=1, SV=0, BP=2, HYB=0, FLAGS=('XLA_TPU_EVENLY_DISTRIBUTE_CRITICAL_NODES',), KL=2, CHL=3, NCL=2, NOFFNDMA=0):
    NB = S // TM
    scope = (lambda n: jax.named_scope(n)) if SCOPES else (lambda n: contextlib.nullcontext())

    def kern(x_hbm, wqkv_hbm, wo_hbm, w1_hbm, w3_hbm, w2_hbm, c_hbm, wmod_hbm, out_hbm,
             x_v, wqkv_v, wp_v, wo_v, wop_v, w1_v, w3_v, w2_v, c_v, wmod_v, kS, vS, qS, oS, x1_v, h_v, out_v, mod_v, scT_v,
             sems, osems):
        cnt = [0]
        def cp(src, dst):
            cnt[0] += 1
            return pltpu.make_async_copy(src, dst, sems.at[cnt[0] - 1])
        def cp2(src, dst, idx):
            return cp(src.at[idx], dst.at[idx])
        KQ = [slice(j * D // KSP, (j + 1) * D // KSP) for j in range(KSP)]
        d_c = cp(c_hbm, c_v)
        d_xa = cp2(x_hbm, x_v, (slice(0, NS * TM), slice(None)))
        d_wv = [cp2(wqkv_hbm, wqkv_v, (ks, slice(2 * D, 3 * D))) for ks in KQ]
        d_m = [[cp2(wmod_hbm, wmod_v, (slice(None), slice(o + ks.start, o + ks.stop))) for o in (D, 0)] for ks in KQ]
        d_xn = cp2(x_hbm, x_v, (slice(NS * TM, (NS + 1) * TM), slice(None)))
        d_xb = cp2(x_hbm, x_v, (slice((NS + 1) * TM, S), slice(None)))
        d_wk = cp2(wqkv_hbm, wqkv_v, (slice(None), slice(D, 2 * D)))
        d_wq = cp2(wqkv_hbm, wqkv_v, (slice(None), slice(0, D)))
        d_wo = cp(wo_hbm, wo_v)
        d_wmb = cp2(wmod_hbm, wmod_v, (slice(None), slice(2 * D, 6 * D)))
        d_w1 = cp(w1_hbm, w1_v)
        d_w3 = cp(w3_hbm, w3_v)
        d_w2 = cp(w2_hbm, w2_v)
        first = [d_c, d_xa]
        for j in range(KSP): first += [d_wv[j]] + d_m[j]
        for d in first + [d_xn, d_xb, d_wk, d_wq, d_wo, d_wmb] + ([] if NOFFNDMA else [d_w1, d_w3, d_w2]):
            d.start()
        kS[:, 0:PAD, :] = jnp.zeros((8, PAD, 128), f32)
        vS[:, 0:PAD, :] = jnp.zeros((8, PAD, 128), f32)

        def nan_gate(vals):
            ok = None
            for v in vals:
                t = pltpu.bitcast(v[0:16, 0:128], i32) != NANBITS
                ok = t if ok is None else jnp.logical_and(ok, t)
            return jnp.where(ok, 0, 1).astype(i32)

        def or_gate(vb, g):
            n, m = vb.shape[0] // 16, vb.shape[1] // 128
            gg = jnp.concatenate([g] * m, axis=1) if m > 1 else g
            gg = jnp.concatenate([gg] * n, axis=0) if n > 1 else gg
            return pltpu.bitcast(pltpu.bitcast(vb, i32) | gg, bf16)

        ptok = []
        def prep_w(t, ks=slice(0, D), gate=None, chained=False):
            out = []
            for g in range(8):
                col = t * D + g * 128
                wb = wqkv_v[ks, col:col + 128]
                if chained and len(ptok) >= PCH: wb = or_gate(wb, nan_gate([ptok[-PCH]]))
                wt = wb.T
                for c in range(8):
                    piece = jnp.concatenate([wt[32 * a + 4 * c:32 * a + 4 * c + 4, :] for a in range(4)], axis=0)
                    if gate is not None and g == 7 and c == 7:
                        piece = or_gate(piece, gate)
                    r0 = t * D + c * 128 + g * 16
                    wp_v[r0:r0 + 16, ks] = piece
                    out.append(piece)
                if chained: ptok.append(piece)
            return out

        def prep_wo(chained=False):
            out = []
            for g in range(8):
                wt = wo_v[g * 128:(g + 1) * 128, :]
                if chained and len(ptok) >= PCH: wt = or_gate(wt, nan_gate([ptok[-PCH]]))
                for c in range(8):
                    piece = jnp.concatenate([wt[32 * a + 4 * c:32 * a + 4 * c + 4, :] for a in range(4)], axis=0)
                    wop_v[c * 128 + g * 16:c * 128 + g * 16 + 16, :] = piece
                    out.append(piece)
                if chained: ptok.append(piece)
            return out

        def two(v):
            return jnp.concatenate([v, v], axis=0)

        def ln_norm(x):
            m = jnp.sum(x, axis=-1, keepdims=True) * (1.0 / D)
            xc = x - m
            v = jnp.sum(xc * xc, axis=-1, keepdims=True) * (1.0 / D)
            rs = lax.rsqrt(v + 1e-5)
            return xc * rs, rs

        def tok_ok(tok):
            return jnp.broadcast_to(tok[0:8], (8, 128)) > -1.0

        ln_tok = []
        def ln1(i):
            for r in range(TM // 16):
                r0 = i * TM + r * 16
                xb = x_v[r0:r0 + 16, :]
                if LNCH1 and len(ln_tok) >= LNCH1:
                    xb = or_gate(xb, jnp.where(tok_ok(ln_tok[-LNCH1]), 0, 1).astype(i32))
                n, rs = ln_norm(xb.astype(f32))
                ln_tok.append(rs)
                h_v[r0:r0 + 16, :] = (n * two(mod_v[:, D:2 * D]) + two(mod_v[:, 0:D])).astype(bf16)

        def ln1_stats(i):
            for r in range(TM // 16):
                r0 = i * TM + r * 16
                n, _ = ln_norm(x_v[r0:r0 + 16, :].astype(f32))
                for c in range(8):
                    qS[c, r0:r0 + 16, :] = n[:, c * 128:(c + 1) * 128]

        def ln1_half(i, ks):
            r0 = i * TM
            for c in range(ks.start // 128, ks.stop // 128):
                cs = slice(c * 128, (c + 1) * 128)
                s1 = jnp.concatenate([mod_v[:, D + c * 128:D + (c + 1) * 128]] * (TM // 8), axis=0)
                sh = jnp.concatenate([mod_v[:, c * 128:(c + 1) * 128]] * (TM // 8), axis=0)
                h_v[r0:r0 + TM, cs] = (qS[c, r0:r0 + TM, :] * s1 + sh).astype(bf16)

        def ln2(i):
            tok = []
            for r in range(TM // 16):
                r0 = i * TM + r * 16
                if not isinstance(r0, int): r0 = pl.multiple_of(r0, 16)
                x = x1_v[pl.ds(r0, 16), :]
                if LNCH and len(tok) >= LNCH:
                    gz = jnp.where(tok_ok(tok[-LNCH]), 0.0, 1.0)
                    x = x + two(jnp.concatenate([gz] * 8, axis=1))
                n, rs = ln_norm(x)
                h_v[pl.ds(r0, 16), :] = (n * two(mod_v[:, 4 * D:5 * D]) + two(mod_v[:, 3 * D:4 * D])).astype(bf16)
                tok.append(rs)
            return tok

        def proj(i, t, dst, pad, ks=None, add=False, gate=None):
            r0 = i * TM
            ks = ks or slice(0, D)
            h = h_v[r0:r0 + TM, ks]
            if gate is not None: h = or_gate(h, gate)
            r = lax.dot_general(h, wp_v[t * D:(t + 1) * D, ks], NT, preferred_element_type=f32)
            for c in range(8):
                rr = r[:, c * 128:(c + 1) * 128]
                if add: rr = rr + dst[c, pad + r0:pad + r0 + TM, :]
                dst[c, pad + r0:pad + r0 + TM, :] = rr

        def proj_mod(i, t, dst, pad, sc, tiles):
            r0 = i * TM
            h = h_v[r0:r0 + TM, :]
            for c in range(8):
                wt = wp_v[t * D + c * 128:t * D + (c + 1) * 128, :]
                j = tiles[c]
                hk = D // 2
                r = lax.dot_general(h[:, :hk], wt[:, :hk], NT, preferred_element_type=f32)
                m = jnp.dot(sc[:, :hk], wmod_v[0:hk, j * 128:(j + 1) * 128], preferred_element_type=f32)
                r = r + lax.dot_general(h[:, hk:], wt[:, hk:], NT, preferred_element_type=f32)
                m = m + jnp.dot(sc[:, hk:], wmod_v[hk:, j * 128:(j + 1) * 128], preferred_element_type=f32)
                dst[c, pad + r0:pad + r0 + TM, :] = r
                m = m[0:8]
                if 4 * 8 <= j < 5 * 8: m = m + 1.0
                mod_v[:, j * 128:(j + 1) * 128] = m

        lane = lax.broadcasted_iota(i32, (R, 128), 1)
        ix1, ix2 = lane ^ 1, lane ^ 2
        chain = []
        held = []
        def att(i):
            ch = CHL if (CHL and NB - 1 - NCL <= i < NB - 1) else CHAIN
            for r in range(TM // R):
                r0 = i * TM + r * R
                qs = QSCALE
                if ch and len(chain) >= ch:
                    qs = jnp.where(chain[-ch] > -1.0, QSCALE, QSCALE * (1 + 2.0 ** -20))
                q = [qS[c, r0:r0 + R, :] * qs for c in range(8)]
                lg = []
                for w in range(W):
                    b0 = PAD + r0 - DIL * w
                    p = q[0] * kS[0, b0:b0 + R, :]
                    for c in range(1, 8):
                        p = p + q[c] * kS[c, b0:b0 + R, :]
                    p = p + jnp.take_along_axis(p, ix1, axis=1)
                    p = p + jnp.take_along_axis(p, ix2, axis=1)
                    if r0 < DIL * w:
                        row = lax.broadcasted_iota(i32, (R, 128), 0) + r0
                        p = jnp.where(row >= DIL * w, p, NEG)
                    lg.append(p)
                mx = jnp.maximum
                m = mx(mx(mx(lg[0], lg[1]), mx(lg[2], lg[3])), mx(mx(lg[4], lg[5]), mx(lg[6], lg[7])))
                e = [jnp.exp2(l - m) for l in lg]
                den = ((e[0] + e[1]) + (e[2] + e[3])) + ((e[4] + e[5]) + (e[6] + e[7]))
                inv = 1.0 / den
                chain.append(e[0])
                for c in range(8):
                    o = e[0] * vS[c, PAD + r0:PAD + r0 + R, :]
                    for w in range(1, W):
                        b0 = PAD + r0 - DIL * w
                        o = o + e[w] * vS[c, b0:b0 + R, :]
                    o = o * inv
                    if PAIR and R == 8:
                        if r % 2 == 0: held.append(o)
                        else: oS[r0 - R:r0 + R, c * 128:(c + 1) * 128] = jnp.concatenate([held.pop(0), o], axis=0).astype(bf16)
                    else:
                        oS[r0:r0 + R, c * 128:(c + 1) * 128] = o.astype(bf16)

        def wo_mm(i):
            r0 = i * TM
            a = jnp.dot(oS[r0:r0 + TM, :], wop_v[...], preferred_element_type=f32)
            ga = mod_v[:, 2 * D:3 * D]
            x1_v[r0:r0 + TM, :] = x_v[r0:r0 + TM, :].astype(f32) + jnp.concatenate([ga] * (TM // 8), axis=0) * a

        def ffn_part(rows, chunks, mid=None):
            h = h_v[rows, :]
            acc = None
            for n, f in enumerate(chunks):
                if mid is not None and n == mid[0]:
                    mid[1]()
                fs = slice(f * TF, (f + 1) * TF)
                g = jnp.dot(h, w1_v[:, fs], preferred_element_type=f32)
                u = jnp.dot(h, w3_v[:, fs], preferred_element_type=f32)
                a = (g * jax.nn.sigmoid(g) * u).astype(bf16)
                y = jnp.dot(a, w2_v[fs, :], preferred_element_type=f32)
                acc = y if acc is None else acc + y
            return acc

        def mod_half(sc, dmas, ks):
            for d in dmas: d.wait()
            for o in (D, 0):
                r = jnp.dot(sc, wmod_v[:, o + ks.start:o + ks.stop], preferred_element_type=f32)[0:8]
                mod_v[:, o + ks.start:o + ks.stop] = r + 1.0 if o == D else r

        with scope('w_xa'):
            d_xa.wait()
        with scope('stats'):
            for i in range(NS): ln1_stats(i)
        with scope('w_wva'):
            d_wv[0].wait()
        with scope('prep_va'):
            prep_w(2, KQ[0])
        d_c.wait()
        cf = c_v[...].astype(f32)
        sc = jnp.broadcast_to((cf * jax.nn.sigmoid(cf)).astype(bf16), (16, D))
        def mod_tile(j, gate=None):
            wb = wmod_v[:, j * 128:(j + 1) * 128]
            if gate is not None: wb = or_gate(wb, gate)
            pr = wb.astype(f32) * scT_v[...]
            a8 = jnp.sum(pr.reshape(D // 8, 8, 128), axis=0)
            m = jnp.broadcast_to(jnp.sum(a8, axis=0, keepdims=True), (8, 128))
            if 8 <= j < 16 or 32 <= j < 40: m = m + 1.0
            mod_v[:, j * 128:(j + 1) * 128] = m
            return a8, m
        if SV or HYB: scT_v[...] = jnp.broadcast_to(sc[0:1].astype(f32), (128, D)).T
        if SV:
            with scope('mod0'):
                mod_half(sc, d_m[0], KQ[0])
            for j in range(KSP):
                with scope(f'RV{j}'):
                    for i in range(NS):
                        if i == BP and j + 1 < KSP:
                            d_wv[j + 1].wait()
                            for d in d_m[j + 1]: d.wait()
                            if j + 2 == KSP: d_xn.wait()
                            prep_w(2, KQ[j + 1])
                            for o in (D, 0):
                                for t in range((o + KQ[j + 1].start) // 128, (o + KQ[j + 1].stop) // 128): mod_tile(t)
                        ln1_half(i, KQ[j])
                        proj(i, 2, vS, PAD, KQ[j], add=j > 0)
                    if j == KSP - 1: ln1(NS)
        else:
          for j in range(KSP):
            with scope(f'mod{j}'):
                if HYB:
                    for d in d_m[j]: d.wait()
                    ks = KQ[j]
                    mod_v[:, ks] = jnp.dot(sc, wmod_v[:, ks], preferred_element_type=f32)[0:8]
                    for t in range((D + ks.start) // 128, (D + ks.stop) // 128): mod_tile(t)
                else:
                    mod_half(sc, d_m[j], KQ[j])
                if j == KSP - 1: d_xn.wait()
            with scope(f'RV{j}'):
                ln1_half(0, KQ[j])
                proj(0, 2, vS, PAD, KQ[j], add=j > 0)
                if j + 1 < KSP:
                    d_wv[j + 1].wait()
                    prep_w(2, KQ[j + 1])
                for i in range(1, NS):
                    ln1_half(i, KQ[j])
                    proj(i, 2, vS, PAD, KQ[j], add=j > 0)
                if j == KSP - 1: ln1(NS)
        with scope('w_xb'):
            d_xb.wait()
        with scope('R3'):
            for i in range(NS + 1, NS + NV1 + 1): ln1(i)
            for i in range(NS, NS + NV1): proj(i, 2, vS, PAD)
            d_wk.wait()
            if EARLYPREP: d_wq.wait(); d_wo.wait()
            for i in range(NS + NV1 + 1, NB): ln1(i)
            prep_w(1, chained=PCH > 0)
            if EARLYPREP: pq = prep_w(0, chained=PCH > 0); pw = prep_wo(chained=PCH > 0)
            for i in range(NS + NV1, NB): proj(i, 2, vS, PAD)
            for i in range(KL):
                gate = None
                if EARLYPREP and TIEP == 1 and i == KL - 1: gate = nan_gate(pw[-8:])
                if EARLYPREP and TIEP == 2: gate = nan_gate(pq if i == 0 else pw)
                proj(i, 1, kS, PAD, gate=gate)
        with scope('w_wq_wo_wmb'):
            if not EARLYPREP: d_wq.wait(); d_wo.wait()
            d_wmb.wait()

        def mod_vpu():
            scT_v[...] = jnp.broadcast_to(sc[0:1].astype(f32), (128, D)).T
            toks = []
            for j in range(16, 48):
                gate = None
                if MODCHN and len(toks) >= MODCHN:
                    t = toks[-MODCHN]
                    gate = jnp.where(t == t, 0, 1).astype(i32)
                a8, m = mod_tile(j, gate)
                toks.append(a8)
                mtok[j] = m

        mtok = {}
        def projm(i, t, dst, pad, tiles):
            if MODV:
                gate = None
                prev = [mtok[j - 8 * MODV] for j in tiles if j - 8 * MODV in mtok]
                if tiles[0] == 40: prev += [mtok[j] for j in range(48 - 8 * MODV, 48)] if MODV else []
                if prev:
                    ok = functools.reduce(jnp.logical_and, [m == m for m in prev])
                    gate = jnp.where(ok, 0, 1).astype(i32)
                proj(i, t, dst, pad, gate=gate)
            else: proj_mod(i, t, dst, pad, sc, tiles)
        with scope('R4'):
            if not EARLYPREP:
                pw = prep_wo()
                prep_w(0, gate=nan_gate(pw) if TIE_WO else None)
            if MODV: mod_vpu()
            projm(KL, 1, kS, PAD, range(16, 24))
            projm(0, 0, qS, 0, range(24, 32))
            ltok = None
            for i in range(1, NB):
                if i == 1:
                    projm(1 + KL, 1, kS, PAD, range(32, 40))
                    projm(1, 0, qS, 0, range(40, 48))
                else:
                    if i + KL < NB:
                        gate = None
                        if TIE_LN and i + KL == TIE_LN:
                            ok = functools.reduce(jnp.logical_and, [tok_ok(t) for t in ltok[-max(LNCH, 1):]])
                            gate = jnp.where(ok, 0, 1).astype(i32)
                        proj(i + KL, 1, kS, PAD, gate=gate)
                    proj(i, 0, qS, 0)
                att(i - 1)
                wo_mm(i - 1)
                if i == 1: ltok = ln2(0)
        with scope('w_ffn'):
            if NOFFNDMA: d_w1.start(); d_w3.start(); d_w2.start()
            d_w1.wait(); d_w3.wait(); d_w2.wait()
        NC = F // TF
        with scope('R5'):
            att(NB - 1)
            ln2(1)
            acc = ffn_part(slice(0, TM), range(0, NA), mid=(NA // 2, lambda: wo_mm(NB - 1)))
            gbt = jnp.concatenate([mod_v[:, 5 * D:6 * D]] * (TM // 8), axis=0)
            x1_v[0:TM, :] = x1_v[0:TM, :] + gbt * acc

        def loopA(i, carry):
            rows = pl.ds(pl.multiple_of(i * TM, TM), TM)
            acc = ffn_part(rows, range(0, NA))
            ln2(jnp.minimum(i + 1, NB - 1))
            gbt = jnp.concatenate([mod_v[:, 5 * D:6 * D]] * (TM // 8), axis=0)
            x1_v[rows, :] = x1_v[rows, :] + gbt * acc
            return carry
        with scope('loopA'):
            lax.fori_loop(1, NB, loopA, 0)

        def loopB(i, carry):
            rows = pl.ds(pl.multiple_of(i * TM, TM), TM)
            acc = ffn_part(rows, range(NA, NC))
            gbt = jnp.concatenate([mod_v[:, 5 * D:6 * D]] * (TM // 8), axis=0)
            out_v[rows, :] = (x1_v[rows, :] + gbt * acc).astype(bf16)
            pltpu.make_async_copy(out_v.at[rows, :], out_hbm.at[rows, :], osems.at[i]).start()
            return carry
        with scope('loopB'):
            lax.fori_loop(0, NB, loopB, 0)
        with scope('tail'):
            for i in range(NB):
                rows = pl.ds(i * TM, TM)
                pltpu.make_async_copy(out_v.at[rows, :], out_hbm.at[rows, :], osems.at[i]).wait()

    V = pltpu.VMEM
    scratch = [V((S, D), bf16), V((D, 3 * D), bf16), V((3 * D, D), bf16), V((D, D), bf16), V((D, D), bf16),
               V((D, F), bf16), V((D, F), bf16), V((F, D), bf16), V((1, D), bf16), V((D, 6 * D), bf16),
               V((8, PAD + S, 128), f32), V((8, PAD + S, 128), f32), V((8, S, 128), f32), V((S, D), bf16),
               V((S, D), f32), V((S, D), bf16), V((S, D), bf16), V((8, 6 * D), f32), V((D, 128), f32),
               pltpu.SemaphoreType.DMA((11 + 3 * KSP,)), pltpu.SemaphoreType.DMA((NB,))]
    call = pl.pallas_call(kern, out_shape=jax.ShapeDtypeStruct((S, D), bf16),
                          in_specs=[pl.BlockSpec(memory_space=pl.ANY)] * 8, out_specs=pl.BlockSpec(memory_space=pl.ANY),
                          scratch_shapes=scratch,
                          compiler_params=pltpu.CompilerParams(vmem_limit_bytes=120 * 1024 * 1024, flags={f: True for f in FLAGS} or None))

    def fn(A_x, A_wqkv, A_wo, B_x, B_w1, B_w3, B_w2, c, w_mod):
        return call(A_x.reshape(S, D), A_wqkv, A_wo, B_w1, B_w3, B_w2, c, w_mod).reshape(1, S, D)
    return fn


_KERNEL = make()


@jax.jit
def pallas_adaLN_cond__sliding_local_dilated__glu_gated_swiglu__prompt_kernel(
    A_x, A_wqkv, A_wo, B_x, B_w1, B_w3, B_w2, c, w_mod
):
    return _KERNEL(A_x, A_wqkv, A_wo, B_x, B_w1, B_w3, B_w2, c, w_mod)
```

```python
import functools, math, contextlib
import jax, jax.numpy as jnp
from jax import lax
from jax.experimental import pallas as pl
from jax.experimental.pallas import tpu as pltpu

S, D, F, H, Dh, W, DIL = 2048, 1024, 3584, 32, 32, 8, 2
PAD = 16
bf16, f32, i32 = jnp.bfloat16, jnp.float32, jnp.int32
QSCALE = Dh ** -0.5 * math.log2(math.e)
NEG = -1e9 * math.log2(math.e)
NT = (((1,), (1,)), ((), ()))
NANBITS = 0x7FC17FC1


def make(TM=256, R=8, TF=512, CHAIN=2, LNCH=2, LNCH1=0, SCOPES=False, NA=4, MODI=2, NS=3,
         TIE_WO=0, TIE_LN=0, TIE_PK=0, KSP=4, NV1=3, EARLYPREP=1, MODV=1, MODCHN=4, PCH=0, TIEP=2, PAIR=1, SV=0, BP=2, HYB=0, GS=0, PCHW=0, MIDP=3, BFLY=1, FLAGS=('XLA_TPU_EVENLY_DISTRIBUTE_CRITICAL_NODES',), KL=2, CHL=3, NCL=2, NOFFNDMA=0):
    NB = S // TM
    scope = (lambda n: jax.named_scope(n)) if SCOPES else (lambda n: contextlib.nullcontext())

    def kern(x_hbm, wqkv_hbm, wo_hbm, w1_hbm, w3_hbm, w2_hbm, c_hbm, wmod_hbm, out_hbm,
             x_v, wqkv_v, wp_v, wo_v, wop_v, w1_v, w3_v, w2_v, c_v, wmod_v, kS, vS, qS, oS, x1_v, h_v, out_v, mod_v, scT_v, g32,
             sems, osems):
        cnt = [0]
        def cp(src, dst):
            cnt[0] += 1
            return pltpu.make_async_copy(src, dst, sems.at[cnt[0] - 1])
        def cp2(src, dst, idx):
            return cp(src.at[idx], dst.at[idx])
        KQ = [slice(j * D // KSP, (j + 1) * D // KSP) for j in range(KSP)]
        d_c = cp(c_hbm, c_v)
        d_xa = cp2(x_hbm, x_v, (slice(0, NS * TM), slice(None)))
        d_wv = [cp2(wqkv_hbm, wqkv_v, (ks, slice(2 * D, 3 * D))) for ks in KQ]
        d_m = [[cp2(wmod_hbm, wmod_v, (slice(None), slice(o + ks.start, o + ks.stop))) for o in (D, 0)] for ks in KQ]
        d_xn = cp2(x_hbm, x_v, (slice(NS * TM, (NS + 1) * TM), slice(None)))
        d_xb = cp2(x_hbm, x_v, (slice((NS + 1) * TM, S), slice(None)))
        d_wk = cp2(wqkv_hbm, wqkv_v, (slice(None), slice(D, 2 * D)))
        d_wq = cp2(wqkv_hbm, wqkv_v, (slice(None), slice(0, D)))
        d_wo = cp(wo_hbm, wo_v)
        d_wmb = cp2(wmod_hbm, wmod_v, (slice(None), slice(2 * D, 6 * D)))
        d_w1 = cp(w1_hbm, w1_v)
        d_w3 = cp(w3_hbm, w3_v)
        d_w2 = cp(w2_hbm, w2_v)
        first = [d_c, d_xa]
        for j in range(KSP): first += [d_wv[j]] + d_m[j]
        for d in first + [d_xn, d_xb, d_wk, d_wq, d_wo, d_wmb] + ([] if NOFFNDMA else [d_w1, d_w3, d_w2]):
            d.start()
        kS[:, 0:PAD, :] = jnp.zeros((8, PAD, 128), f32)
        vS[:, 0:PAD, :] = jnp.zeros((8, PAD, 128), f32)

        def nan_gate(vals):
            ok = None
            for v in vals:
                t = pltpu.bitcast(v[0:16, 0:128], i32) != NANBITS
                ok = t if ok is None else jnp.logical_and(ok, t)
            return jnp.where(ok, 0, 1).astype(i32)

        def or_gate(vb, g):
            n, m = vb.shape[0] // 16, vb.shape[1] // 128
            gg = jnp.concatenate([g] * m, axis=1) if m > 1 else g
            gg = jnp.concatenate([gg] * n, axis=0) if n > 1 else gg
            return pltpu.bitcast(pltpu.bitcast(vb, i32) | gg, bf16)

        ptok = []
        gslot = [0]
        sub8 = lax.broadcasted_iota(i32, (8, 128), 0)
        def regroup_bfly(wt, dst, row_of, col0, gate_last=None):
            n = wt.shape[1]
            w32 = pltpu.bitcast(wt, i32)
            sub = lax.broadcasted_iota(i32, (8, n), 0)
            lo4, even = sub < 4, (sub & 2) == 0
            rot = lambda v, k: pltpu.roll(v, k, 0)
            res = {}
            for half in range(2):
                A = [w32[8 * (2 * a + half):8 * (2 * a + half) + 8, :] for a in range(4)]
                B0 = jnp.where(lo4, A[0], rot(A[2], 4)); B2 = jnp.where(lo4, rot(A[0], 4), A[2])
                B1 = jnp.where(lo4, A[1], rot(A[3], 4)); B3 = jnp.where(lo4, rot(A[1], 4), A[3])
                res[4 * half + 0] = jnp.where(even, B0, rot(B1, 2)); res[4 * half + 1] = jnp.where(even, rot(B0, 6), B1)
                res[4 * half + 2] = jnp.where(even, B2, rot(B3, 2)); res[4 * half + 3] = jnp.where(even, rot(B2, 6), B3)
            out = []
            for c in range(8):
                piece = pltpu.bitcast(res[c], bf16)
                if gate_last is not None and c == 7: piece = or_gate(piece, gate_last)
                r0 = row_of(c)
                dst[r0:r0 + 16, col0:col0 + n] = piece
                out.append(piece)
            return out

        def regroup(wt, dst, row_of, col0, gate_last=None):
            if BFLY: return regroup_bfly(wt, dst, row_of, col0, gate_last)
            sl = gslot[0] % GS; gslot[0] += 1
            w32 = pltpu.bitcast(wt, i32)
            nb = wt.shape[1] // 128
            for j in range(nb): g32[sl, j] = w32[:, j * 128:(j + 1) * 128]
            out = []
            for c in range(8):
                cols = []
                for j in range(nb):
                    v = g32[sl, j, 42 + 2 * c:50 + 2 * c, :]
                    for a in (2, 1, 0):
                        v = jnp.where(sub8 < 2 * a + 2, g32[sl, j, 14 * a + 2 * c:14 * a + 2 * c + 8, :], v)
                    cols.append(v)
                piece = pltpu.bitcast(jnp.concatenate(cols, axis=1), bf16)
                if gate_last is not None and c == 7: piece = or_gate(piece, gate_last)
                r0 = row_of(c)
                dst[r0:r0 + 16, col0:col0 + nb * 128] = piece
                out.append(piece)
            return out
        def prep_w(t, ks=slice(0, D), gate=None, chained=False):
            out = []
            for g in range(8):
                col = t * D + g * 128
                wb = wqkv_v[ks, col:col + 128]
                if chained and len(ptok) >= PCH: wb = or_gate(wb, nan_gate([ptok[-PCH]]))
                wt = wb.T
                if GS or BFLY:
                    out += regroup(wt, wp_v, lambda c: t * D + c * 128 + g * 16, ks.start, gate if g == 7 else None)
                    if chained: ptok.append(out[-1])
                    continue
                for c in range(8):
                    piece = jnp.concatenate([wt[32 * a + 4 * c:32 * a + 4 * c + 4, :] for a in range(4)], axis=0)
                    if gate is not None and g == 7 and c == 7:
                        piece = or_gate(piece, gate)
                    r0 = t * D + c * 128 + g * 16
                    wp_v[r0:r0 + 16, ks] = piece
                    out.append(piece)
                if chained: ptok.append(piece)
            return out

        def prep_wo(chained=False, start_tok=None):
            out = []
            for g in range(8):
                wt = wo_v[g * 128:(g + 1) * 128, :]
                if chained and len(ptok) >= PCH: wt = or_gate(wt, nan_gate([ptok[-PCH]]))
                if PCHW and start_tok is not None and g < PCHW: wt = or_gate(wt, start_tok)
                if PCHW and g >= PCHW: wt = or_gate(wt, nan_gate([out[8 * (g - PCHW) + 7]]))
                if GS or BFLY:
                    out += regroup(wt, wop_v, lambda c: c * 128 + g * 16, 0)
                    if chained: ptok.append(out[-1])
                    continue
                for c in range(8):
                    piece = jnp.concatenate([wt[32 * a + 4 * c:32 * a + 4 * c + 4, :] for a in range(4)], axis=0)
                    wop_v[c * 128 + g * 16:c * 128 + g * 16 + 16, :] = piece
                    out.append(piece)
                if chained: ptok.append(piece)
            return out

        def two(v):
            return jnp.concatenate([v, v], axis=0)

        def ln_norm(x):
            m = jnp.sum(x, axis=-1, keepdims=True) * (1.0 / D)
            xc = x - m
            v = jnp.sum(xc * xc, axis=-1, keepdims=True) * (1.0 / D)
            rs = lax.rsqrt(v + 1e-5)
            return xc * rs, rs

        def tok_ok(tok):
            return jnp.broadcast_to(tok[0:8], (8, 128)) > -1.0

        ln_tok = []
        def ln1(i):
            for r in range(TM // 16):
                r0 = i * TM + r * 16
                xb = x_v[r0:r0 + 16, :]
                if LNCH1 and len(ln_tok) >= LNCH1:
                    xb = or_gate(xb, jnp.where(tok_ok(ln_tok[-LNCH1]), 0, 1).astype(i32))
                n, rs = ln_norm(xb.astype(f32))
                ln_tok.append(rs)
                h_v[r0:r0 + 16, :] = (n * two(mod_v[:, D:2 * D]) + two(mod_v[:, 0:D])).astype(bf16)

        def ln1_stats(i):
            for r in range(TM // 16):
                r0 = i * TM + r * 16
                n, _ = ln_norm(x_v[r0:r0 + 16, :].astype(f32))
                for c in range(8):
                    qS[c, r0:r0 + 16, :] = n[:, c * 128:(c + 1) * 128]

        def ln1_half(i, ks):
            r0 = i * TM
            for c in range(ks.start // 128, ks.stop // 128):
                cs = slice(c * 128, (c + 1) * 128)
                s1 = jnp.concatenate([mod_v[:, D + c * 128:D + (c + 1) * 128]] * (TM // 8), axis=0)
                sh = jnp.concatenate([mod_v[:, c * 128:(c + 1) * 128]] * (TM // 8), axis=0)
                h_v[r0:r0 + TM, cs] = (qS[c, r0:r0 + TM, :] * s1 + sh).astype(bf16)

        def ln2(i):
            tok = []
            for r in range(TM // 16):
                r0 = i * TM + r * 16
                if not isinstance(r0, int): r0 = pl.multiple_of(r0, 16)
                x = x1_v[pl.ds(r0, 16), :]
                if LNCH and len(tok) >= LNCH:
                    gz = jnp.where(tok_ok(tok[-LNCH]), 0.0, 1.0)
                    x = x + two(jnp.concatenate([gz] * 8, axis=1))
                n, rs = ln_norm(x)
                h_v[pl.ds(r0, 16), :] = (n * two(mod_v[:, 4 * D:5 * D]) + two(mod_v[:, 3 * D:4 * D])).astype(bf16)
                tok.append(rs)
            return tok

        def proj(i, t, dst, pad, ks=None, add=False, gate=None):
            r0 = i * TM
            ks = ks or slice(0, D)
            h = h_v[r0:r0 + TM, ks]
            if gate is not None: h = or_gate(h, gate)
            r = lax.dot_general(h, wp_v[t * D:(t + 1) * D, ks], NT, preferred_element_type=f32)
            for c in range(8):
                rr = r[:, c * 128:(c + 1) * 128]
                if add: rr = rr + dst[c, pad + r0:pad + r0 + TM, :]
                dst[c, pad + r0:pad + r0 + TM, :] = rr

        def proj_mod(i, t, dst, pad, sc, tiles):
            r0 = i * TM
            h = h_v[r0:r0 + TM, :]
            for c in range(8):
                wt = wp_v[t * D + c * 128:t * D + (c + 1) * 128, :]
                j = tiles[c]
                hk = D // 2
                r = lax.dot_general(h[:, :hk], wt[:, :hk], NT, preferred_element_type=f32)
                m = jnp.dot(sc[:, :hk], wmod_v[0:hk, j * 128:(j + 1) * 128], preferred_element_type=f32)
                r = r + lax.dot_general(h[:, hk:], wt[:, hk:], NT, preferred_element_type=f32)
                m = m + jnp.dot(sc[:, hk:], wmod_v[hk:, j * 128:(j + 1) * 128], preferred_element_type=f32)
                dst[c, pad + r0:pad + r0 + TM, :] = r
                m = m[0:8]
                if 4 * 8 <= j < 5 * 8: m = m + 1.0
                mod_v[:, j * 128:(j + 1) * 128] = m

        lane = lax.broadcasted_iota(i32, (R, 128), 1)
        ix1, ix2 = lane ^ 1, lane ^ 2
        chain = []
        held = []
        def att(i):
            ch = CHL if (CHL and NB - 1 - NCL <= i < NB - 1) else CHAIN
            for r in range(TM // R):
                r0 = i * TM + r * R
                qs = QSCALE
                if ch and len(chain) >= ch:
                    qs = jnp.where(chain[-ch] > -1.0, QSCALE, QSCALE * (1 + 2.0 ** -20))
                q = [qS[c, r0:r0 + R, :] * qs for c in range(8)]
                lg = []
                for w in range(W):
                    b0 = PAD + r0 - DIL * w
                    p = q[0] * kS[0, b0:b0 + R, :]
                    for c in range(1, 8):
                        p = p + q[c] * kS[c, b0:b0 + R, :]
                    p = p + jnp.take_along_axis(p, ix1, axis=1)
                    p = p + jnp.take_along_axis(p, ix2, axis=1)
                    if r0 < DIL * w:
                        row = lax.broadcasted_iota(i32, (R, 128), 0) + r0
                        p = jnp.where(row >= DIL * w, p, NEG)
                    lg.append(p)
                mx = jnp.maximum
                m = mx(mx(mx(lg[0], lg[1]), mx(lg[2], lg[3])), mx(mx(lg[4], lg[5]), mx(lg[6], lg[7])))
                e = [jnp.exp2(l - m) for l in lg]
                den = ((e[0] + e[1]) + (e[2] + e[3])) + ((e[4] + e[5]) + (e[6] + e[7]))
                inv = 1.0 / den
                chain.append(e[0])
                for c in range(8):
                    o = e[0] * vS[c, PAD + r0:PAD + r0 + R, :]
                    for w in range(1, W):
                        b0 = PAD + r0 - DIL * w
                        o = o + e[w] * vS[c, b0:b0 + R, :]
                    o = o * inv
                    if PAIR and R == 8:
                        if r % 2 == 0: held.append(o)
                        else: oS[r0 - R:r0 + R, c * 128:(c + 1) * 128] = jnp.concatenate([held.pop(0), o], axis=0).astype(bf16)
                    else:
                        oS[r0:r0 + R, c * 128:(c + 1) * 128] = o.astype(bf16)

        def wo_mm(i):
            r0 = i * TM
            a = jnp.dot(oS[r0:r0 + TM, :], wop_v[...], preferred_element_type=f32)
            ga = mod_v[:, 2 * D:3 * D]
            x1_v[r0:r0 + TM, :] = x_v[r0:r0 + TM, :].astype(f32) + jnp.concatenate([ga] * (TM // 8), axis=0) * a

        def ffn_part(rows, chunks, mid=None):
            h = h_v[rows, :]
            acc = None
            for n, f in enumerate(chunks):
                if mid is not None and n == mid[0]:
                    mid[1]()
                fs = slice(f * TF, (f + 1) * TF)
                g = jnp.dot(h, w1_v[:, fs], preferred_element_type=f32)
                u = jnp.dot(h, w3_v[:, fs], preferred_element_type=f32)
                a = (g * jax.nn.sigmoid(g) * u).astype(bf16)
                y = jnp.dot(a, w2_v[fs, :], preferred_element_type=f32)
                acc = y if acc is None else acc + y
            return acc

        def mod_half(sc, dmas, ks):
            for d in dmas: d.wait()
            for o in (D, 0):
                r = jnp.dot(sc, wmod_v[:, o + ks.start:o + ks.stop], preferred_element_type=f32)[0:8]
                mod_v[:, o + ks.start:o + ks.stop] = r + 1.0 if o == D else r

        with scope('w_xa'):
            d_xa.wait()
        with scope('stats'):
            for i in range(NS): ln1_stats(i)
        with scope('w_wva'):
            d_wv[0].wait()
        with scope('prep_va'):
            prep_w(2, KQ[0])
        d_c.wait()
        cf = c_v[...].astype(f32)
        sc = jnp.broadcast_to((cf * jax.nn.sigmoid(cf)).astype(bf16), (16, D))
        def mod_tile(j, gate=None):
            wb = wmod_v[:, j * 128:(j + 1) * 128]
            if gate is not None: wb = or_gate(wb, gate)
            pr = wb.astype(f32) * scT_v[...]
            a8 = jnp.sum(pr.reshape(D // 8, 8, 128), axis=0)
            m = jnp.broadcast_to(jnp.sum(a8, axis=0, keepdims=True), (8, 128))
            if 8 <= j < 16 or 32 <= j < 40: m = m + 1.0
            mod_v[:, j * 128:(j + 1) * 128] = m
            return a8, m
        if SV or HYB: scT_v[...] = jnp.broadcast_to(sc[0:1].astype(f32), (128, D)).T
        if SV:
            with scope('mod0'):
                mod_half(sc, d_m[0], KQ[0])
            for j in range(KSP):
                with scope(f'RV{j}'):
                    for i in range(NS):
                        if i == BP and j + 1 < KSP:
                            d_wv[j + 1].wait()
                            for d in d_m[j + 1]: d.wait()
                            if j + 2 == KSP: d_xn.wait()
                            prep_w(2, KQ[j + 1])
                            for o in (D, 0):
                                for t in range((o + KQ[j + 1].start) // 128, (o + KQ[j + 1].stop) // 128): mod_tile(t)
                        ln1_half(i, KQ[j])
                        proj(i, 2, vS, PAD, KQ[j], add=j > 0)
                    if j == KSP - 1: ln1(NS)
        else:
          for j in range(KSP):
            with scope(f'mod{j}'):
                if HYB:
                    for d in d_m[j]: d.wait()
                    ks = KQ[j]
                    mod_v[:, ks] = jnp.dot(sc, wmod_v[:, ks], preferred_element_type=f32)[0:8]
                    for t in range((D + ks.start) // 128, (D + ks.stop) // 128): mod_tile(t)
                else:
                    mod_half(sc, d_m[j], KQ[j])
                if j == KSP - 1: d_xn.wait()
            with scope(f'RV{j}'):
                ln1_half(0, KQ[j])
                proj(0, 2, vS, PAD, KQ[j], add=j > 0)
                if j + 1 < KSP:
                    d_wv[j + 1].wait()
                    prep_w(2, KQ[j + 1])
                for i in range(1, NS):
                    ln1_half(i, KQ[j])
                    proj(i, 2, vS, PAD, KQ[j], add=j > 0)
                if j == KSP - 1: ln1(NS)
        with scope('w_xb'):
            d_xb.wait()
        with scope('R3'):
            for i in range(NS + 1, NS + NV1 + 1): ln1(i)
            for i in range(NS, NS + NV1): proj(i, 2, vS, PAD)
            d_wk.wait()
            if EARLYPREP: d_wq.wait(); d_wo.wait()
            for i in range(NS + NV1 + 1, NB): ln1(i)
            pk = prep_w(1, chained=PCH > 0)
            if EARLYPREP: pq = prep_w(0, chained=PCH > 0); pw = prep_wo(chained=PCH > 0, start_tok=nan_gate(pk[-1:]))
            for i in range(NS + NV1, NB): proj(i, 2, vS, PAD)
            for i in range(KL):
                gate = None
                if EARLYPREP and TIEP == 1 and i == KL - 1: gate = nan_gate(pw[-8:])
                if EARLYPREP and TIEP == 2: gate = nan_gate(pq if i == 0 else pw)
                proj(i, 1, kS, PAD, gate=gate)
        with scope('w_wq_wo_wmb'):
            if not EARLYPREP: d_wq.wait(); d_wo.wait()
            d_wmb.wait()

        def mod_vpu():
            scT_v[...] = jnp.broadcast_to(sc[0:1].astype(f32), (128, D)).T
            toks = []
            for j in range(16, 48):
                gate = None
                if MODCHN and len(toks) >= MODCHN:
                    t = toks[-MODCHN]
                    gate = jnp.where(t == t, 0, 1).astype(i32)
                a8, m = mod_tile(j, gate)
                toks.append(a8)
                mtok[j] = m

        mtok = {}
        def projm(i, t, dst, pad, tiles):
            if MODV:
                gate = None
                prev = [mtok[j - 8 * MODV] for j in tiles if j - 8 * MODV in mtok]
                if tiles[0] == 40: prev += [mtok[j] for j in range(48 - 8 * MODV, 48)] if MODV else []
                if prev:
                    ok = functools.reduce(jnp.logical_and, [m == m for m in prev])
                    gate = jnp.where(ok, 0, 1).astype(i32)
                proj(i, t, dst, pad, gate=gate)
            else: proj_mod(i, t, dst, pad, sc, tiles)
        with scope('R4'):
            if not EARLYPREP:
                pw = prep_wo()
                prep_w(0, gate=nan_gate(pw) if TIE_WO else None)
            if MODV: mod_vpu()
            projm(KL, 1, kS, PAD, range(16, 24))
            projm(0, 0, qS, 0, range(24, 32))
            ltok = None
            for i in range(1, NB):
                if i == 1:
                    projm(1 + KL, 1, kS, PAD, range(32, 40))
                    projm(1, 0, qS, 0, range(40, 48))
                else:
                    if i + KL < NB:
                        gate = None
                        if TIE_LN and i + KL == TIE_LN:
                            ok = functools.reduce(jnp.logical_and, [tok_ok(t) for t in ltok[-max(LNCH, 1):]])
                            gate = jnp.where(ok, 0, 1).astype(i32)
                        proj(i + KL, 1, kS, PAD, gate=gate)
                    proj(i, 0, qS, 0)
                att(i - 1)
                wo_mm(i - 1)
                if i == 1: ltok = ln2(0)
        with scope('w_ffn'):
            if NOFFNDMA: d_w1.start(); d_w3.start(); d_w2.start()
            d_w1.wait(); d_w3.wait(); d_w2.wait()
        NC = F // TF
        with scope('R5'):
            att(NB - 1)
            ln2(1)
            acc = ffn_part(slice(0, TM), range(0, NA), mid=(MIDP, lambda: wo_mm(NB - 1)))
            gbt = jnp.concatenate([mod_v[:, 5 * D:6 * D]] * (TM // 8), axis=0)
            x1_v[0:TM, :] = x1_v[0:TM, :] + gbt * acc

        def loopA(i, carry):
            rows = pl.ds(pl.multiple_of(i * TM, TM), TM)
            acc = ffn_part(rows, range(0, NA))
            ln2(jnp.minimum(i + 1, NB - 1))
            gbt = jnp.concatenate([mod_v[:, 5 * D:6 * D]] * (TM // 8), axis=0)
            x1_v[rows, :] = x1_v[rows, :] + gbt * acc
            return carry
        with scope('loopA'):
            lax.fori_loop(1, NB, loopA, 0)

        def loopB(i, carry):
            rows = pl.ds(pl.multiple_of(i * TM, TM), TM)
            acc = ffn_part(rows, range(NA, NC))
            gbt = jnp.concatenate([mod_v[:, 5 * D:6 * D]] * (TM // 8), axis=0)
            out_v[rows, :] = (x1_v[rows, :] + gbt * acc).astype(bf16)
            pltpu.make_async_copy(out_v.at[rows, :], out_hbm.at[rows, :], osems.at[i]).start()
            return carry
        with scope('loopB'):
            lax.fori_loop(0, NB, loopB, 0)
        with scope('tail'):
            for i in range(NB):
                rows = pl.ds(i * TM, TM)
                pltpu.make_async_copy(out_v.at[rows, :], out_hbm.at[rows, :], osems.at[i]).wait()

    V = pltpu.VMEM
    scratch = [V((S, D), bf16), V((D, 3 * D), bf16), V((3 * D, D), bf16), V((D, D), bf16), V((D, D), bf16),
               V((D, F), bf16), V((D, F), bf16), V((F, D), bf16), V((1, D), bf16), V((D, 6 * D), bf16),
               V((8, PAD + S, 128), f32), V((8, PAD + S, 128), f32), V((8, S, 128), f32), V((S, D), bf16),
               V((S, D), f32), V((S, D), bf16), V((S, D), bf16), V((8, 6 * D), f32), V((D, 128), f32), V((max(GS, 1), 8, 64, 128), i32),
               pltpu.SemaphoreType.DMA((11 + 3 * KSP,)), pltpu.SemaphoreType.DMA((NB,))]
    call = pl.pallas_call(kern, out_shape=jax.ShapeDtypeStruct((S, D), bf16),
                          in_specs=[pl.BlockSpec(memory_space=pl.ANY)] * 8, out_specs=pl.BlockSpec(memory_space=pl.ANY),
                          scratch_shapes=scratch,
                          compiler_params=pltpu.CompilerParams(vmem_limit_bytes=120 * 1024 * 1024, flags={f: True for f in FLAGS} or None))

    def fn(A_x, A_wqkv, A_wo, B_x, B_w1, B_w3, B_w2, c, w_mod):
        return call(A_x.reshape(S, D), A_wqkv, A_wo, B_w1, B_w3, B_w2, c, w_mod).reshape(1, S, D)
    return fn


_KERNEL = make()


@jax.jit
def pallas_adaLN_cond__sliding_local_dilated__glu_gated_swiglu__prompt_kernel(
    A_x, A_wqkv, A_wo, B_x, B_w1, B_w3, B_w2, c, w_mod
):
    return _KERNEL(A_x, A_wqkv, A_wo, B_x, B_w1, B_w3, B_w2, c, w_mod)
```

```python
import functools
import math

import jax
import jax.numpy as jnp
from jax import lax
from jax.experimental import pallas as pl
from jax.experimental.pallas import tpu as pltpu

S, D, F, DH, W, DIL = 2048, 1024, 3584, 32, 8, 2
TM = 256
NB = S // TM
R = 8
PAD = 16
TF = 512
NA = 4
NS = 3
KSP = 4
KL = 2
bf16, f32, i32 = jnp.bfloat16, jnp.float32, jnp.int32
LOG2E = math.log2(math.e)
QSCALE = DH ** -0.5 * LOG2E
NEG = -1e9 * LOG2E
NT = (((1,), (1,)), ((), ()))
NANBITS = 0x7FC17FC1


def _two(v):
    return jnp.concatenate([v, v], axis=0)


def _rows(v):
    return jnp.concatenate([v] * (TM // 8), axis=0)


def _nan_gate(vals):
    ok = None
    for v in vals:
        t = pltpu.bitcast(v[0:16, 0:128], i32) != NANBITS
        ok = t if ok is None else jnp.logical_and(ok, t)
    return jnp.where(ok, 0, 1).astype(i32)


def _or_gate(vb, g):
    n, m = vb.shape[0] // 16, vb.shape[1] // 128
    gg = jnp.concatenate([g] * m, axis=1) if m > 1 else g
    gg = jnp.concatenate([gg] * n, axis=0) if n > 1 else gg
    return pltpu.bitcast(pltpu.bitcast(vb, i32) | gg, bf16)


def _ln_norm(x):
    m = jnp.sum(x, axis=-1, keepdims=True) * (1.0 / D)
    xc = x - m
    v = jnp.sum(xc * xc, axis=-1, keepdims=True) * (1.0 / D)
    rs = lax.rsqrt(v + 1e-5)
    return xc * rs, rs


def _regroup(wt, dst, row_of, col0):
    n = wt.shape[1]
    w32 = pltpu.bitcast(wt, i32)
    sub = lax.broadcasted_iota(i32, (8, n), 0)
    lo4, even = sub < 4, (sub & 2) == 0
    rot = lambda v, k: pltpu.roll(v, k, 0)
    res = {}
    for half in range(2):
        a = [w32[8 * (2 * h + half):8 * (2 * h + half) + 8, :] for h in range(4)]
        b0 = jnp.where(lo4, a[0], rot(a[2], 4))
        b2 = jnp.where(lo4, rot(a[0], 4), a[2])
        b1 = jnp.where(lo4, a[1], rot(a[3], 4))
        b3 = jnp.where(lo4, rot(a[1], 4), a[3])
        res[4 * half + 0] = jnp.where(even, b0, rot(b1, 2))
        res[4 * half + 1] = jnp.where(even, rot(b0, 6), b1)
        res[4 * half + 2] = jnp.where(even, b2, rot(b3, 2))
        res[4 * half + 3] = jnp.where(even, rot(b2, 6), b3)
    out = []
    for c in range(8):
        piece = pltpu.bitcast(res[c], bf16)
        r0 = row_of(c)
        dst[r0:r0 + 16, col0:col0 + n] = piece
        out.append(piece)
    return out


def _kernel(x_hbm, wqkv_hbm, wo_hbm, w1_hbm, w3_hbm, w2_hbm, c_hbm, wmod_hbm, out_hbm,
            x_v, wqkv_v, wp_v, wo_v, wop_v, w1_v, w3_v, w2_v, c_v, wmod_v,
            kS, vS, qS, oS, x1_v, h_v, out_v, mod_v, scT_v, sems, osems):
    count = [0]

    def cp(src, dst, idx=None):
        if idx is not None:
            src, dst = src.at[idx], dst.at[idx]
        count[0] += 1
        return pltpu.make_async_copy(src, dst, sems.at[count[0] - 1])

    every = slice(None)
    KQ = [slice(j * D // KSP, (j + 1) * D // KSP) for j in range(KSP)]
    d_c = cp(c_hbm, c_v)
    d_xa = cp(x_hbm, x_v, (slice(0, NS * TM), every))
    d_wv = [cp(wqkv_hbm, wqkv_v, (ks, slice(2 * D, 3 * D))) for ks in KQ]
    d_m = [[cp(wmod_hbm, wmod_v, (every, slice(o + ks.start, o + ks.stop))) for o in (D, 0)] for ks in KQ]
    d_xn = cp(x_hbm, x_v, (slice(NS * TM, (NS + 1) * TM), every))
    d_xb = cp(x_hbm, x_v, (slice((NS + 1) * TM, S), every))
    d_wk = cp(wqkv_hbm, wqkv_v, (every, slice(D, 2 * D)))
    d_wq = cp(wqkv_hbm, wqkv_v, (every, slice(0, D)))
    d_wo = cp(wo_hbm, wo_v)
    d_wmb = cp(wmod_hbm, wmod_v, (every, slice(2 * D, 6 * D)))
    d_w1 = cp(w1_hbm, w1_v)
    d_w3 = cp(w3_hbm, w3_v)
    d_w2 = cp(w2_hbm, w2_v)
    order = [d_c, d_xa]
    for j in range(KSP):
        order += [d_wv[j]] + d_m[j]
    for d in order + [d_xn, d_xb, d_wk, d_wq, d_wo, d_wmb, d_w1, d_w3, d_w2]:
        d.start()
    kS[:, 0:PAD, :] = jnp.zeros((8, PAD, 128), f32)
    vS[:, 0:PAD, :] = jnp.zeros((8, PAD, 128), f32)

    def prep_w(t, ks=slice(0, D)):
        out = []
        for g in range(8):
            col = t * D + g * 128
            wt = wqkv_v[ks, col:col + 128].T
            out += _regroup(wt, wp_v, lambda c: t * D + c * 128 + g * 16, ks.start)
        return out

    def prep_wo():
        out = []
        for g in range(8):
            out += _regroup(wo_v[g * 128:(g + 1) * 128, :], wop_v, lambda c: c * 128 + g * 16, 0)
        return out

    def ln1(i):
        for r in range(TM // 16):
            r0 = i * TM + r * 16
            n, _ = _ln_norm(x_v[r0:r0 + 16, :].astype(f32))
            h_v[r0:r0 + 16, :] = (n * _two(mod_v[:, D:2 * D]) + _two(mod_v[:, 0:D])).astype(bf16)

    def ln1_stats(i):
        for r in range(TM // 16):
            r0 = i * TM + r * 16
            n, _ = _ln_norm(x_v[r0:r0 + 16, :].astype(f32))
            for c in range(8):
                qS[c, r0:r0 + 16, :] = n[:, c * 128:(c + 1) * 128]

    def ln1_part(i, ks):
        r0 = i * TM
        for c in range(ks.start // 128, ks.stop // 128):
            s1 = _rows(mod_v[:, D + c * 128:D + (c + 1) * 128])
            sh = _rows(mod_v[:, c * 128:(c + 1) * 128])
            h_v[r0:r0 + TM, c * 128:(c + 1) * 128] = (qS[c, r0:r0 + TM, :] * s1 + sh).astype(bf16)

    def ln2(i):
        tok = []
        for r in range(TM // 16):
            r0 = i * TM + r * 16
            if not isinstance(r0, int):
                r0 = pl.multiple_of(r0, 16)
            x = x1_v[pl.ds(r0, 16), :]
            if len(tok) >= 2:
                zero = jnp.where(jnp.broadcast_to(tok[-2][0:8], (8, 128)) > -1.0, 0.0, 1.0)
                x = x + _two(jnp.concatenate([zero] * 8, axis=1))
            n, rs = _ln_norm(x)
            h_v[pl.ds(r0, 16), :] = (n * _two(mod_v[:, 4 * D:5 * D]) + _two(mod_v[:, 3 * D:4 * D])).astype(bf16)
            tok.append(rs)

    def proj(i, t, dst, pad, ks=slice(0, D), add=False, gate=None):
        r0 = i * TM
        h = h_v[r0:r0 + TM, ks]
        if gate is not None:
            h = _or_gate(h, gate)
        r = lax.dot_general(h, wp_v[t * D:(t + 1) * D, ks], NT, preferred_element_type=f32)
        for c in range(8):
            rr = r[:, c * 128:(c + 1) * 128]
            if add:
                rr = rr + dst[c, pad + r0:pad + r0 + TM, :]
            dst[c, pad + r0:pad + r0 + TM, :] = rr

    lane = lax.broadcasted_iota(i32, (R, 128), 1)
    ix1, ix2 = lane ^ 1, lane ^ 2
    chain, held = [], []

    def att(i):
        depth = 3 if NB - 3 <= i < NB - 1 else 2
        for r in range(TM // R):
            r0 = i * TM + r * R
            qs = QSCALE
            if len(chain) >= depth:
                qs = jnp.where(chain[-depth] > -1.0, QSCALE, QSCALE * (1 + 2.0 ** -20))
            q = [qS[c, r0:r0 + R, :] * qs for c in range(8)]
            lg = []
            for w in range(W):
                b0 = PAD + r0 - DIL * w
                p = q[0] * kS[0, b0:b0 + R, :]
                for c in range(1, 8):
                    p = p + q[c] * kS[c, b0:b0 + R, :]
                p = p + jnp.take_along_axis(p, ix1, axis=1)
                p = p + jnp.take_along_axis(p, ix2, axis=1)
                if r0 < DIL * w:
                    row = lax.broadcasted_iota(i32, (R, 128), 0) + r0
                    p = jnp.where(row >= DIL * w, p, NEG)
                lg.append(p)
            mx = jnp.maximum
            m = mx(mx(mx(lg[0], lg[1]), mx(lg[2], lg[3])), mx(mx(lg[4], lg[5]), mx(lg[6], lg[7])))
            e = [jnp.exp2(l - m) for l in lg]
            den = ((e[0] + e[1]) + (e[2] + e[3])) + ((e[4] + e[5]) + (e[6] + e[7]))
            inv = 1.0 / den
            chain.append(e[0])
            for c in range(8):
                o = e[0] * vS[c, PAD + r0:PAD + r0 + R, :]
                for w in range(1, W):
                    b0 = PAD + r0 - DIL * w
                    o = o + e[w] * vS[c, b0:b0 + R, :]
                o = o * inv
                if r % 2 == 0:
                    held.append(o)
                else:
                    oS[r0 - R:r0 + R, c * 128:(c + 1) * 128] = jnp.concatenate([held.pop(0), o], axis=0).astype(bf16)

    def wo_mm(i):
        r0 = i * TM
        a = jnp.dot(oS[r0:r0 + TM, :], wop_v[...], preferred_element_type=f32)
        x1_v[r0:r0 + TM, :] = x_v[r0:r0 + TM, :].astype(f32) + _rows(mod_v[:, 2 * D:3 * D]) * a

    def ffn_part(rows, chunks, mid=None):
        h = h_v[rows, :]
        acc = None
        for n, f in enumerate(chunks):
            if mid is not None and n == mid[0]:
                mid[1]()
            fs = slice(f * TF, (f + 1) * TF)
            g = jnp.dot(h, w1_v[:, fs], preferred_element_type=f32)
            u = jnp.dot(h, w3_v[:, fs], preferred_element_type=f32)
            a = (g * jax.nn.sigmoid(g) * u).astype(bf16)
            y = jnp.dot(a, w2_v[fs, :], preferred_element_type=f32)
            acc = y if acc is None else acc + y
        return acc

    d_xa.wait()
    for i in range(NS):
        ln1_stats(i)
    d_wv[0].wait()
    prep_w(2, KQ[0])
    d_c.wait()
    cf = c_v[...].astype(f32)
    sc = jnp.broadcast_to((cf * jax.nn.sigmoid(cf)).astype(bf16), (16, D))
    for j, ks in enumerate(KQ):
        for d in d_m[j]:
            d.wait()
        for o in (D, 0):
            r = jnp.dot(sc, wmod_v[:, o + ks.start:o + ks.stop], preferred_element_type=f32)[0:8]
            mod_v[:, o + ks.start:o + ks.stop] = r + 1.0 if o == D else r
        if j == KSP - 1:
            d_xn.wait()
        ln1_part(0, ks)
        proj(0, 2, vS, PAD, ks, add=j > 0)
        if j + 1 < KSP:
            d_wv[j + 1].wait()
            prep_w(2, KQ[j + 1])
        for i in range(1, NS):
            ln1_part(i, ks)
            proj(i, 2, vS, PAD, ks, add=j > 0)
        if j == KSP - 1:
            ln1(NS)

    d_xb.wait()
    for i in range(NS + 1, NB):
        ln1(i)
    for i in range(NS, NS + 3):
        proj(i, 2, vS, PAD)
    d_wk.wait()
    d_wq.wait()
    d_wo.wait()
    prep_w(1)
    pq = prep_w(0)
    pw = prep_wo()
    for i in range(NS + 3, NB):
        proj(i, 2, vS, PAD)
    for i in range(KL):
        proj(i, 1, kS, PAD, gate=_nan_gate(pq if i == 0 else pw))

    d_wmb.wait()
    scT_v[...] = jnp.broadcast_to(sc[0:1].astype(f32), (128, D)).T
    toks, mtok = [], {}
    for j in range(16, 48):
        wb = wmod_v[:, j * 128:(j + 1) * 128]
        if len(toks) >= 4:
            t = toks[-4]
            wb = _or_gate(wb, jnp.where(t == t, 0, 1).astype(i32))
        a8 = jnp.sum((wb.astype(f32) * scT_v[...]).reshape(D // 8, 8, 128), axis=0)
        m = jnp.broadcast_to(jnp.sum(a8, axis=0, keepdims=True), (8, 128))
        if 32 <= j < 40:
            m = m + 1.0
        mod_v[:, j * 128:(j + 1) * 128] = m
        toks.append(a8)
        mtok[j] = m

    def after(tiles):
        ok = functools.reduce(jnp.logical_and, [mtok[j] == mtok[j] for j in tiles])
        return jnp.where(ok, 0, 1).astype(i32)

    proj(KL, 1, kS, PAD)
    proj(0, 0, qS, 0, gate=after(range(16, 24)))
    for i in range(1, NB):
        if i + KL < NB:
            proj(i + KL, 1, kS, PAD, gate=after(range(24, 32)) if i == 1 else None)
        proj(i, 0, qS, 0, gate=after(range(32, 48)) if i == 1 else None)
        att(i - 1)
        wo_mm(i - 1)
        if i == 1:
            ln2(0)

    d_w1.wait()
    d_w3.wait()
    d_w2.wait()
    att(NB - 1)
    ln2(1)
    acc = ffn_part(slice(0, TM), range(NA), mid=(3, lambda: wo_mm(NB - 1)))
    x1_v[0:TM, :] = x1_v[0:TM, :] + _rows(mod_v[:, 5 * D:6 * D]) * acc

    def loop_a(i, carry):
        rows = pl.ds(pl.multiple_of(i * TM, TM), TM)
        acc = ffn_part(rows, range(NA))
        ln2(jnp.minimum(i + 1, NB - 1))
        x1_v[rows, :] = x1_v[rows, :] + _rows(mod_v[:, 5 * D:6 * D]) * acc
        return carry

    lax.fori_loop(1, NB, loop_a, 0)

    def loop_b(i, carry):
        rows = pl.ds(pl.multiple_of(i * TM, TM), TM)
        acc = ffn_part(rows, range(NA, F // TF))
        out_v[rows, :] = (x1_v[rows, :] + _rows(mod_v[:, 5 * D:6 * D]) * acc).astype(bf16)
        pltpu.make_async_copy(out_v.at[rows, :], out_hbm.at[rows, :], osems.at[i]).start()
        return carry

    lax.fori_loop(0, NB, loop_b, 0)
    for i in range(NB):
        rows = pl.ds(i * TM, TM)
        pltpu.make_async_copy(out_v.at[rows, :], out_hbm.at[rows, :], osems.at[i]).wait()


def _build():
    V = pltpu.VMEM
    scratch = [
        V((S, D), bf16), V((D, 3 * D), bf16), V((3 * D, D), bf16), V((D, D), bf16), V((D, D), bf16),
        V((D, F), bf16), V((D, F), bf16), V((F, D), bf16), V((1, D), bf16), V((D, 6 * D), bf16),
        V((8, PAD + S, 128), f32), V((8, PAD + S, 128), f32), V((8, S, 128), f32), V((S, D), bf16),
        V((S, D), f32), V((S, D), bf16), V((S, D), bf16), V((8, 6 * D), f32), V((D, 128), f32),
        pltpu.SemaphoreType.DMA((11 + 3 * KSP,)), pltpu.SemaphoreType.DMA((NB,)),
    ]
    return pl.pallas_call(
        _kernel,
        out_shape=jax.ShapeDtypeStruct((S, D), bf16),
        in_specs=[pl.BlockSpec(memory_space=pl.ANY)] * 8,
        out_specs=pl.BlockSpec(memory_space=pl.ANY),
        scratch_shapes=scratch,
        compiler_params=pltpu.CompilerParams(
            vmem_limit_bytes=120 * 1024 * 1024,
            flags={"XLA_TPU_EVENLY_DISTRIBUTE_CRITICAL_NODES": True},
        ),
    )


@jax.jit
def pallas_adaLN_cond__sliding_local_dilated__glu_gated_swiglu__prompt_kernel(
    A_x, A_wqkv, A_wo, B_x, B_w1, B_w3, B_w2, c, w_mod
):
    del B_x
    out = _build()(A_x.reshape(S, D), A_wqkv, A_wo, B_w1, B_w3, B_w2, c, w_mod)
    return out.reshape(1, S, D)
```
